```python
import os as _os
_os.environ.setdefault("JAX_PLATFORMS", "cpu")
import jax
import jax.numpy as jnp

def _softmax(x, axis=-1):
    return jax.nn.softmax(x, axis=axis)
def _gelu(x):
    return jax.nn.gelu(x, approximate=True)
def _silu(x):
    return jax.nn.silu(x)
def _sigmoid(x):
    return jax.nn.sigmoid(x)
def _layernorm(x, axis=-1, eps=1e-5):
    m = jnp.mean(x, axis=axis, keepdims=True)
    v = jnp.var(x, axis=axis, keepdims=True)
    return (x - m) / jnp.sqrt(v + eps)
def _scatter_add(tgt, idx, src, axis=0):
    return tgt.at[idx].add(src)
def _segment_sum(src, seg, n):
    return jax.ops.segment_sum(src, seg, n)
class _Rng:
    def __init__(self, key):
        self._k = key
    def _next(self):
        self._k, sub = jax.random.split(self._k)
        return sub
    def normal(self, shape):
        return jax.random.normal(self._next(), shape, dtype=jnp.bfloat16)
    def randint(self, lo, hi, shape):
        return jax.random.randint(self._next(), shape, lo, hi, dtype=jnp.int32)
    def uniform(self, shape, lo=0.0, hi=1.0):
        return jax.random.uniform(self._next(), shape, jnp.bfloat16, lo, hi)
    def permutation(self, n):
        return jax.random.permutation(self._next(), n)


kernel_name = 'sequential_preLN__sliding_block__mixer_channel_mlp__prompt'

def setup_inputs():
    _rng = _Rng(jax.random.key(int.from_bytes(__import__("os").urandom(4), "little")))
    _w = (lambda a: (lambda t: t.astype(jnp.bfloat16) if jnp.issubdtype(t.dtype, jnp.floating) else t)(jnp.asarray(a)))
    def _A_setup():
        B, S, D = 1, 2048, 1024
        return {
            "x": _w((lambda *s: _rng.normal(s) * 0.05)(B, S, D)),
            "wqkv": _w((lambda *s: _rng.normal(s) * 0.05)(D, 3 * D)),
            "wo": _w((lambda *s: _rng.normal(s) * 0.05)(D, D)),
        }
    _A_in = _A_setup()

    def _B_setup():
        B, S, D, F = 1, 2048, 1024, 3584
        return {
            "x": _w((lambda *s: _rng.normal(s) * 0.05)(B, S, D)),
            "w1": _w((lambda *s: _rng.normal(s) * 0.8)(D, F) * (D ** -0.5)),
            "b1": _w((lambda *s: _rng.normal(s) * 0.8)(F)),
            "w2": _w((lambda *s: _rng.normal(s) * 0.8)(F, D) * (F ** -0.5)),
            "b2": _w((lambda *s: _rng.normal(s) * 0.05)(D)),
        }
    _B_in = _B_setup()

    return {
        "A_x": _A_in["x"],
        "A_wqkv": _A_in["wqkv"],
        "A_wo": _A_in["wo"],
        "B_x": _B_in["x"],
        "B_w1": _B_in["w1"],
        "B_b1": _B_in["b1"],
        "B_w2": _B_in["w2"],
        "B_b2": _B_in["b2"],
    }

def reference(A_x, A_wqkv, A_wo, B_x, B_w1, B_b1, B_w2, B_b2):
    def _A_ref(x, wqkv, wo):
        B, S, D = x.shape
        H = 32; Dh = D // H; W = 256
        qkv = (lambda x, *d: x.transpose(*d))((x @ wqkv).reshape(B, S, 3, H, Dh), 2, 0, 3, 1, 4)
        q, k, v = qkv[0], qkv[1], qkv[2]
        scores = jnp.einsum("bhqd,bhkd->bhqk", q, k) * (Dh ** -0.5)
        idx = jnp.arange(S)
        mask = (idx[:, None] - idx[None, :] >= 0) & (idx[:, None] - idx[None, :] < W)
        scores = jnp.where(mask[None, None], scores, -1e9)
        p = _softmax(scores, axis=-1)
        o = jnp.einsum("bhqk,bhkd->bhqd", p, v)
        return (lambda x, *d: x.transpose(*d))(o, 0, 2, 1, 3).reshape(B, S, D) @ wo

    def _B_ref(x, w1, b1, w2, b2):
        y = _layernorm(x, axis=-1)
        h = _gelu(jnp.einsum("bsd,df->bsf", y, w1) + b1)
        return jnp.einsum("bsf,fd->bsd", h, w2) + b2

    x = A_x
    h = x + _A_ref(_layernorm(x, axis=-1), A_wqkv, A_wo)
    h2 = h + _B_ref(_layernorm(h, axis=-1), B_w1, B_b1, B_w2, B_b2)
    return h2
```

```python
import functools
import math

import jax
import jax.numpy as jnp
import numpy as np
from jax import lax
import jax.experimental.pallas as pl
import jax.experimental.pallas.tpu as pltpu

S, D, F = 2048, 1024, 3584
H, DH, W = 32, 32, 256
EPS = 1e-5
TM1 = 256
TM3 = 256
FC = 512
NG_UNROLL = 8
BF = jnp.bfloat16
F32 = jnp.float32


def _ln(x):
    m = jnp.mean(x, axis=-1, keepdims=True)
    xc = x - m
    v = jnp.mean(xc * xc, axis=-1, keepdims=True)
    return xc * lax.rsqrt(v + EPS)


def _gelu(z):
    c0 = math.sqrt(2.0 / math.pi)
    c1 = c0 * 0.044715
    u = z * z * c1 + c0
    t = jnp.tanh(z * u)
    hz = 0.5 * z
    return hz * t + hz


def _dot(a, b):
    return jnp.dot(a, b, preferred_element_type=F32)


def _dot_nt(a, b):
    return lax.dot_general(a, b, (((1,), (1,)), ((), ())), preferred_element_type=F32)


def _kernel(x_hbm, wqkv_hbm, wo_hbm, w1_hbm, b1_ref, w2_hbm, b2_ref, o_hbm,
            x_s, wqkv_s, wo_s, w1_s, w2_s, q_s, k_s, vt_s, a_s, out_s, sem_x, sem_w, sem_o):
    n1 = S // TM1
    n3 = S // TM3

    def x_copy(i):
        return pltpu.make_async_copy(x_hbm.at[pl.ds(i * TM1, TM1)], x_s.at[pl.ds(i * TM1, TM1)], sem_x.at[i])

    wq = [pltpu.make_async_copy(wqkv_hbm.at[:, pl.ds(j * D, D)], wqkv_s.at[:, pl.ds(j * D, D)], sem_w.at[j]) for j in range(3)]
    c_wo = pltpu.make_async_copy(wo_hbm, wo_s, sem_w.at[3])
    c_w1 = pltpu.make_async_copy(w1_hbm, w1_s, sem_w.at[4])
    c_w2 = pltpu.make_async_copy(w2_hbm, w2_s, sem_w.at[5])
    x_copy(0).start()
    for c in wq:
        c.start()
    for i in range(1, n1):
        x_copy(i).start()
    c_wo.start()
    c_w1.start()
    c_w2.start()

    k_s[pl.ds(0, W), :] = jnp.zeros((W, D), BF)
    vt_s[0] = jnp.zeros((D, 128), BF)
    vt_s[1] = jnp.zeros((D, 128), BF)

    for c in wq:
        c.wait()

    qscale = (DH ** -0.5) * math.log2(math.e)

    def p1(i, carry):
        x_copy(i).wait()
        r0 = pl.multiple_of(i * TM1, TM1)
        xn = _ln(x_s[pl.ds(r0, TM1), :].astype(F32)).astype(BF)
        q = _dot(xn, wqkv_s[:, 0:D])
        q_s[pl.ds(r0, TM1), :] = (q * qscale).astype(BF)
        k = _dot(xn, wqkv_s[:, D:2 * D])
        k_s[pl.ds(r0 + W, TM1), :] = k.astype(BF)
        v = _dot(xn, wqkv_s[:, 2 * D:3 * D])
        for j in range(TM1 // 128):
            vt_s[i * (TM1 // 128) + 2 + j] = v[j * 128:(j + 1) * 128, :].T.astype(BF)
        return carry

    lax.fori_loop(0, n1, p1, 0)

    lane = lax.broadcasted_iota(jnp.int32, (32, 128), 1)
    row = lax.broadcasted_iota(jnp.int32, (32, 128), 0)
    top_valid = row > (lane % 32)
    lane_grp = lane // 32

    def p2(sb, carry):
        r0 = pl.multiple_of(sb * 128, 128)
        for g in range(H // 4):
            cols = pl.ds(g * 128, 128)
            ps = []
            ls = []
            for t in range(4):
                qt = q_s[pl.ds(r0 + 32 * t, 32), cols]
                zero = jnp.zeros_like(qt)
                rhs = jnp.concatenate([jnp.where(lane_grp == (c ^ t), qt, zero) for c in range(4)], axis=0)
                kw = k_s[pl.ds(r0 + 32 * t, 288), cols]
                s = _dot_nt(kw, rhs)
                kpos = lax.broadcasted_iota(jnp.int32, (288, 128), 0) + (r0 + 32 * t - W)
                s = jnp.where(kpos >= 0, s, -1e30)
                edge = jnp.where(top_valid, s[0:32], s[256:288])
                sm = jnp.concatenate([edge, s[32:256]], axis=0)
                m = jnp.max(sm, axis=0, keepdims=True)
                p = jnp.exp2(sm - m)
                l = jnp.sum(p, axis=0, keepdims=True)
                pe = p[0:32]
                parts = []
                if t > 0:
                    parts.append(jnp.zeros((32 * t, 128), BF))
                parts += [jnp.where(top_valid, pe, 0.0).astype(BF), p[32:256].astype(BF), jnp.where(top_valid, 0.0, pe).astype(BF)]
                if t < 3:
                    parts.append(jnp.zeros((32 * (3 - t), 128), BF))
                ps.append(jnp.concatenate(parts, axis=0))
                ls.append(l)

            def butterfly(v):
                ln_ = lax.broadcasted_iota(jnp.int32, v[0].shape, 1)
                b0 = (ln_ & 32) == 0
                b1 = (ln_ & 64) == 0
                u = [jnp.where(b0, v[i], v[i ^ 1]) for i in range(4)]
                return [jnp.where(b1, u[i], u[i ^ 2]) for i in range(4)]

            ph = butterfly(ps)
            lh = butterfly(ls)
            outs = []
            for h in range(4):
                frows = pl.ds(g * 128 + 32 * h, 32)
                vt = jnp.concatenate([vt_s[sb + j, frows, :] for j in range(3)], axis=1)
                o = _dot(vt, ph[h])
                outs.append(o * (1.0 / lh[h]))
            ot = jnp.concatenate(outs, axis=0).T
            ob = butterfly([ot[32 * c:32 * (c + 1)] for c in range(4)])
            a_s[pl.ds(r0, 128), cols] = jnp.concatenate(ob, axis=0).astype(BF)
        return carry

    lax.fori_loop(0, S // 128, p2, 0)

    c_wo.wait()
    c_w1.wait()
    c_w2.wait()

    def o_copy(i):
        return pltpu.make_async_copy(out_s.at[pl.ds(i * TM3, TM3)], o_hbm.at[pl.ds(i * TM3, TM3)], sem_o.at[i])

    def p3(i, carry):
        r0 = pl.multiple_of(i * TM3, TM3)
        h = x_s[pl.ds(r0, TM3), :].astype(F32) + _dot(a_s[pl.ds(r0, TM3), :], wo_s[...])
        y = _ln(_ln(h)).astype(BF)
        acc = h + b2_ref[...].astype(F32)
        for j in range(F // FC):
            z = _dot(y, w1_s[:, j * FC:(j + 1) * FC]) + b1_ref[:, j * FC:(j + 1) * FC].astype(F32)
            acc = acc + _dot(_gelu(z).astype(BF), w2_s[j * FC:(j + 1) * FC, :])
        out_s[pl.ds(r0, TM3), :] = acc.astype(BF)
        o_copy(i).start()
        return carry

    lax.fori_loop(0, n3, p3, 0)
    for i in range(n3):
        o_copy(i).wait()


@jax.jit
def pallas_sequential_preLN__sliding_block__mixer_channel_mlp__prompt_kernel(
        A_x, A_wqkv, A_wo, B_x, B_w1, B_b1, B_w2, B_b2):
    del B_x
    any_spec = pl.BlockSpec(memory_space=pl.ANY)
    vmem_spec = pl.BlockSpec(memory_space=pltpu.VMEM)
    out = pl.pallas_call(
        _kernel,
        out_shape=jax.ShapeDtypeStruct((S, D), BF),
        in_specs=[any_spec, any_spec, any_spec, any_spec, vmem_spec, any_spec, vmem_spec],
        out_specs=any_spec,
        scratch_shapes=[
            pltpu.VMEM((S, D), BF), pltpu.VMEM((D, 3 * D), BF), pltpu.VMEM((D, D), BF),
            pltpu.VMEM((D, F), BF), pltpu.VMEM((F, D), BF),
            pltpu.VMEM((S, D), BF), pltpu.VMEM((S + W, D), BF), pltpu.VMEM((S // 128 + 2, D, 128), BF),
            pltpu.VMEM((S, D), BF), pltpu.VMEM((S, D), BF),
            pltpu.SemaphoreType.DMA((S // TM1,)), pltpu.SemaphoreType.DMA((6,)), pltpu.SemaphoreType.DMA((S // TM3,)),
        ],
        compiler_params=pltpu.CompilerParams(vmem_limit_bytes=110 << 20),
        name="fused_block",
    )(A_x.reshape(S, D), A_wqkv, A_wo, B_w1, B_b1.reshape(1, F), B_w2, B_b2.reshape(1, D))
    return out.reshape(1, S, D)
```

```python
import math

import jax
import jax.numpy as jnp
from jax import lax
import jax.experimental.pallas as pl
import jax.experimental.pallas.tpu as pltpu

S, D, F = 2048, 1024, 3584
DH, W = 32, 256
EPS = 1e-5
TB = 512
NB = S // TB
NP = F // 512
PART = 3
NBT = NB
BLK0 = 0
NPT = NP
NEARLY = 6
KEARLY = 3
EXP_GAP = 26
T_DELAY = 400
LNX_GAP = 390
LNX_GAP0 = 215
WA_GAP00 = 18
WA_GAP0 = 18
WA_GAP1 = 130
ATT0 = 32
LNX_DELAY = 200
LNH_GAP = 114
LNH_GAP_LAST = 118
LNH_DELAY = 100
LNH_GROUP = 4
LNX_GROUP = 2
XLU_STEP = 200
YSLOTS = 6
FUSE_LN = False
GELU_GAP = 48
GELU_GAP_LAST = 56
WGT_GAP = 60
W1_GAP = 56
O_GAP = 200
W1_EARLY = (0, 1, 2, 3, 4)
W1_LATE = ((), (), (), (), (), (), ())
W1_TAIL = (5, 6)
W1_GAP0 = 19
SPLITS = ("b1", "b2", "b3", "w1", "n1", "n3", "n5", "w2", "m1")
BF, F32, I32 = jnp.bfloat16, jnp.float32, jnp.int32
ORDER1 = (1, 3, 2, 4, 5, 0, 6)
ORDER2 = ((1, 3, 2, 4, 5, 0, 6), (6, 1, 3, 2, 4, 5, 0))

GS = (math.sqrt(2.0 / math.pi) * 0.044715) ** (1.0 / 3.0)
GK = math.sqrt(2.0 / math.pi) / GS


def _ln(x, scales=None):
    m = jnp.mean(x, axis=-1, keepdims=True)
    yield
    xc = x - m
    v = jnp.mean(xc * xc, axis=-1, keepdims=True)
    yield
    r = lax.rsqrt(v + EPS)
    if FUSE_LN and scales == (GS,):
        r = r * lax.rsqrt(v * r * r + EPS)
    if scales is None:
        return xc * r
    n = x.shape[1] // len(scales)
    rs = {c: r * c for c in scales}
    return _cat([xc[:, n * i:n * (i + 1)] * rs[c] for i, c in enumerate(scales)], 1)


def _dot(a, b):
    return jnp.dot(a, b, preferred_element_type=F32)


def _dot_nt(a, b):
    return lax.dot_general(a, b, (((1,), (1,)), ((), ())), preferred_element_type=F32)


def _cat(xs, axis):
    return xs[0] if len(xs) == 1 else jnp.concatenate(xs, axis=axis)


def _words(x):
    return pltpu.bitcast(x.astype(BF), I32)


def _halves(w):
    return pltpu.bitcast(w, BF)


def _lhs7(a):
    (a11, a12), (a21, a22) = a
    return [a11 + a22, a21 + a22, a11, a22, a11 + a12, a21 - a11, a12 - a22]


def _rhs7(p, b):
    if p == 0:
        return b(0, 0) + b(1, 1)
    if p == 1:
        return b(0, 0)
    if p == 2:
        return b(0, 1) - b(1, 1)
    if p == 3:
        return b(1, 0) - b(0, 0)
    if p == 4:
        return b(1, 1)
    if p == 5:
        return b(0, 0) + b(0, 1)
    return b(1, 0) + b(1, 1)


_TERMS = {(0, 0): {0: 1, 3: 1, 4: -1, 6: 1}, (0, 1): {2: 1, 4: 1},
          (1, 0): {1: 1, 3: 1}, (1, 1): {0: 1, 1: -1, 2: 1, 5: 1}}


def _out4(m, i, j, order):
    acc = None
    for p in reversed(order):
        sign = _TERMS[i, j].get(p)
        if sign:
            acc = m(p) if acc is None else (acc + m(p) if sign > 0 else acc - m(p))
    return acc


def _last(i, j, order):
    return [p for p in order if p in _TERMS[i, j]][-1]


def _rhs_sub(tile, p):
    return {(i, j): _rhs7(p, lambda hi, hj: tile(2 * hi + i, 2 * hj + j)) for i in range(2) for j in range(2)}


_ROW = (1.0, math.sqrt(3.0), math.sqrt(3.0), 3.0)
_COL = _ROW[::-1]
BAL1 = (0, 1, 2, 4, 6, 3, 5)
BAL2 = ((1, 2, 4, 6, 3, 5, 0), BAL1)
BAL_TURN = ((1, 2, 3, 5, 0, 4, 6), ((0, 0), (0, 1)))
STD_TURN = (ORDER1, ((0, 0), (1, 1)))


def _bal_lhs7(a):
    (a11, a12), (a21, a22) = a
    s, t = a11 + a22, a12 + a21
    return [s, a11 - a12, a11 + a12, s - t, a12 - a22, s + t, a12 + a22]


def _bal_rhs7(b):
    (b11, b12), (b21, b22) = b
    s, t = b11 + b22, b12 + b21
    return [s + s, b12 - b22, b12 + b22, b11 + b12, s + t, b11 - b12, s - t]


def _bal_out(m, order):
    c12, e = m[1] + m[2], m[1] - m[2]
    c21 = (c12 - (m[4] + m[6])) + (m[5] - m[3])
    if order[0] == 0:
        d = e + m[0]
        return [[d + (m[4] - m[6]), c12], [c21, d - (m[3] + m[5])]]
    return [[(e + (m[4] - m[6])) + m[0], c12], [c21, (e - (m[3] + m[5])) + m[0]]]


def _nested(f, a):
    low = {(hi, hj): f([[a[2 * hi + i][2 * hj + j] for j in range(2)] for i in range(2)])
           for hi in range(2) for hj in range(2)}
    return {(p, q): v for q in range(7)
            for p, v in enumerate(f([[low[hi, hj][q] for hj in range(2)] for hi in range(2)]))}


def _lane_bits(shape):
    lane = lax.broadcasted_iota(I32, shape, 1)
    return (lane & 32) == 0, (lane & 64) == 0


def _butterfly(v):
    b0, b1 = _lane_bits(v[0].shape)
    u = [jnp.where(b0, v[i], v[i ^ 1]) for i in range(4)]
    return [jnp.where(b1, u[i], u[i ^ 2]) for i in range(4)]


class _Pacer:
    def __init__(self):
        lane = lax.broadcasted_iota(I32, (8, 128), 1)
        self.never = lane * lane == 2
        self.now = 0.0
        self.mark = None
        self.free = {}
        self.events = []
        self.dues = []

    def after(self, value):
        return value if self.mark is None else jnp.where(self.never, self.mark, value)

    def due(self, value, delay):
        self.dues.append((self.now + delay, pltpu.bitcast(value, I32)))

    def add(self, lane, gap, job, tag=None):
        t = max(self.now, self.free.get(lane, 0.0))
        self.free[lane] = t + gap
        self.events.append((t, tag or lane, job))
        self.events.sort(key=lambda e: e[0])

    def stepwise(self, tag, steps):
        def job():
            if next(steps, self) is not self:
                self.events.append((self.now + XLU_STEP, tag, job))
                self.events.sort(key=lambda e: e[0])
        return job

    def tick(self, r, cycles):
        n = r.shape[0] // 8
        for i in range(n):
            self.now += cycles / n
            while self.events and self.events[0][0] <= self.now:
                self.mark = r[8 * i:8 * (i + 1), :128]
                self.events.pop(0)[2]()
        self.mark = None

    def flush(self, tag):
        while any(e[1] == tag for e in self.events):
            i = [e[1] for e in self.events].index(tag)
            self.now, now = self.events[i][0], self.now
            self.events.pop(i)[2]()
            self.now = now

    def dot(self, words, rhs, cycles, last=True):
        for t, v in self.dues:
            if t < self.now + cycles:
                i = 8 * max(0, int((t - self.now) * (words.shape[0] // 8) / cycles))
                row = _cat([jnp.where(self.never, v, words[i:i + 8, c:c + 128])
                            for c in range(0, words.shape[1], 128)], 1)
                words = _cat(([words[:i]] if i else []) + [row] + ([words[i + 8:]] if i + 8 < words.shape[0] else []), 0)
        r = _dot(_halves(words), rhs)
        if last:
            self.dues = [d for d in self.dues if d[0] >= self.now + cycles]
            self.tick(r, cycles)
        return r


class _Words:
    def __init__(self, pool, start, rows, tiles):
        self.pool, self.start, self.rows = pool, start, rows // 2
        self.end = start + self.rows * ((tiles + 1) // 2)
        assert self.end <= pool.shape[0]

    def _window(self, r0, n, t):
        r = self.start + (t // 2) * self.rows + r0 // 2
        return slice(r, r + n), slice(128 * (t % 2), 128 * (t % 2 + 1))

    def get(self, r0, r1, t0, t1=None):
        return _cat([self.pool[self._window(r0, (r1 - r0) // 2, t)] for t in range(t0, t1 or t0 + 1)], 1)

    def put_words(self, r0, t, w):
        self.pool[self._window(r0, w.shape[0], t)] = w

    def put(self, r0, t0, x):
        for t in range(x.shape[1] // 128):
            self.put_words(r0, t0 + t, _words(x[:, 128 * t:128 * (t + 1)]))


def _interleave(a, na, b, nb):
    ia = ib = 0
    while ia < na or ib < nb:
        if ib >= nb or (ia < na and ia * nb <= ib * na):
            next(a)
            ia += 1
        else:
            next(b)
            ib += 1


def _kernel(x_hbm, wqkv_hbm, wo_hbm, w1_hbm, b1_hbm, w2_hbm, b2_hbm, o_hbm,
            x_s, wo_s, w1_s, w2_s, b1_s, b2_s, e_s, y_s, o_s, p_pool, ya_pool, wb_pool, pool, sem_in, sem_out):
    HB = TB // 2
    QB = TB // 4
    pacer = _Pacer()
    every = slice(None)
    sems = iter(range(sem_in.shape[0]))

    def copy(src, dst):
        return pltpu.make_async_copy(src, dst, sem_in.at[next(sems)])

    def wqkv_copy(m, c0, n):
        return copy(wqkv_hbm.at[:, pl.ds(m * D + c0, n)], w2_s.at[pl.ds(m * D, D), pl.ds(c0, n)])

    def x_copy(r0, r1):
        return copy(x_hbm.at[pl.ds(r0, r1 - r0)], x_s.at[pl.ds(r0, r1 - r0)])

    stages = [[x_copy(r, r + QB)] for r in range(0, TB, QB)] + [
        [wqkv_copy(0, 0, 256)],
        [wqkv_copy(0, 256, 256)],
        [wqkv_copy(1, 0, 512), wqkv_copy(0, 512, 512)],
        [wqkv_copy(2, 0, 512), wqkv_copy(1, 512, 512)],
        [wqkv_copy(2, 512, 512), x_copy(TB, 2 * TB)],
        [x_copy(2 * TB, S)],
        [copy(wo_hbm, wo_s), copy(b1_hbm, b1_s), copy(b2_hbm, b2_s), copy(w1_hbm, w1_s)],
    ]
    w2_copy = copy(w2_hbm, w2_s)
    for stage in stages:
        for c in stage:
            c.start()

    def landed():
        for c in stages.pop(0):
            c.wait()

    lane = lax.broadcasted_iota(I32, (32, 128), 1)
    row = lax.broadcasted_iota(I32, (32, 128), 0)
    top_valid = row > (lane & 31)
    lane16 = lax.broadcasted_iota(I32, (16, 128), 1)
    row16 = lax.broadcasted_iota(I32, (16, 128), 0)
    top_words = (jnp.where(2 * row16 > (lane16 & 31), 0xFFFF, 0)
                 | jnp.where(2 * row16 + 1 > (lane16 & 31), -0x10000, 0))
    zero = pl.multiple_of((lane16 * lane16)[0, 0], 8)
    for buf in (p_pool, ya_pool, wb_pool, pool):
        buf[pl.ds(zero, 8), 0:128] = jnp.zeros((8, 128), I32)
    y_s[pl.ds(zero, 8), 0:128] = jnp.zeros((8, 128), F32)
    o_s[pl.ds(zero, 8), 0:128] = jnp.zeros((8, 128), F32)
    p_s = _Words(p_pool, 0, 3 * 384, 4)
    ya_s = _Words(ya_pool, 0, 49 * S // 4, 2)
    wb_s = _Words(wb_pool, 0, 49 * 256, NP)
    ga_s = _Words(pool, 0, 25 * S // 4, 2 * NP)
    xa_s = _Words(pool, 0, 2 * 49 * QB, 2)
    oa_s = _Words(pool, xa_s.end, 7 * S // 2, 4)
    q_s = _Words(pool, oa_s.end, 2 * TB, 8)
    k_s = _Words(pool, q_s.end, S, 8)
    vt_s = _Words(pool, k_s.end, D, S // 128)
    wa_s = _Words(pool, vt_s.end, 49 * 256, 6)
    wc_s = _Words(pool, wa_s.end, 7 * 512, 4)
    xn_s = _Words(pool, wa_s.end, TB, 8)

    def ga_at(p, q, n):
        k = (7 * p + q) * NP + n
        return k // (2 * NP) * (S // 4), k % (2 * NP)

    def split(name):
        if name in SPLITS:
            @pl.when(zero != 0)
            def _():
                e_s[0:8, 0:128] = jnp.zeros((8, 128), I32)
                p_pool[0:8, 0:128] = jnp.zeros((8, 128), I32)

    qscale = (DH ** -0.5) * math.log2(math.e)

    def after_first(x):
        return _cat([pacer.after(x[:, :128]), x[:, 128:]], 1)

    def queue_operands(lane, gap, tag, lhs7, turn, tied, tile, put):
        low = {}
        for q in turn:
            def job(q=q):
                if not low:
                    t = [[tile(a, b) for b in range(4)] for a in range(4)]
                    for hi in range(2):
                        for hj in range(2):
                            low[hi, hj] = lhs7([[t[2 * hi + i][2 * hj + k] for k in range(2)] for i in range(2)])
                v = {k: low[k][q] for k in low}
                for k in tied:
                    v[k] = _cat([pacer.after(v[k][:8]), v[k][8:]], 0)
                for p, w in enumerate(lhs7([[v[a, b] for b in range(2)] for a in range(2)])):
                    put(p, q, w)
            pacer.add(lane, gap, job, tag)

    slots = [0]

    def queue_rows(lane, blk, gap, delay, group, normed, scheme, dest, row0):
        for r in range(0, QB, 16):
            y0 = 64 * (slots[0] % YSLOTS)
            slots[0] += 1
            first = {}
            for i in range(4):
                for rr in (0, 8):
                    def steps(r=r, i=i, rr=rr, y0=y0, first=first):
                        y = yield from normed(i, r + rr)
                        for b in range(blk + 1):
                            pacer.flush(("y", b, y0))
                        y_s[y0 + 16 * i + rr:y0 + 16 * i + rr + 8, :] = y
                        first[0] = first[0] + y[:, :128] if first else y[:, :128]
                        if (2 * i + rr // 8 + 1) % group == 0:
                            pacer.due(first.pop(0), delay)
                        if i == 3 and rr:
                            pacer.free[lane + "c"] = max(pacer.free.get(lane + "c", 0), pacer.now + delay + 50)
                            for c in range(2):
                                queue_operands(
                                    lane + "c", gap * 8 / 15, ("y", blk, y0), *scheme,
                                    lambda a, b, c=c: y_s[y0 + 16 * a:y0 + 16 * (a + 1), 256 * b + 128 * c:256 * b + 128 * (c + 1)],
                                    lambda p, q, w, c=c: dest.put(row0(7 * p + q) + r, c, w))
                    pacer.add(lane, gap, pacer.stepwise((lane, blk), steps()), (lane, blk))

    def finish_rows(lane, upto):
        for blk in range(upto + 1):
            pacer.flush((lane, blk))
            for i in range(YSLOTS):
                pacer.flush(("y", blk, 64 * i))

    def queue_x(blk):
        def normed(i, r):
            r0 = blk * TB + i * QB + r
            return _ln(after_first(x_s[r0:r0 + 8, :].astype(F32)), [_ROW[i] * c for c in _COL])
        queue_rows("x", blk, LNX_GAP if blk > 1 else LNX_GAP0, LNX_DELAY, LNX_GROUP, normed, (_bal_lhs7,) + BAL_TURN, xa_s,
                   lambda k: (blk % 2 * 49 + k) * QB)

    def queue_wa(j, m, gap):
        for r in range(0, 256, 16):
            def tile(a, b, r=r):
                r0, c0 = m * D + 256 * a + r, 512 * j + 256 * (b // 2)
                w = w2_s[r0:r0 + 16, c0:c0 + 256].astype(F32)
                return w[:, 128 * (b % 2):128 * (b % 2 + 1)] * (_ROW[a] * _COL[b])
            queue_operands("w", gap, ("wa", j, m), _bal_rhs7, *BAL_TURN, tile,
                           lambda p, q, w, r=r: wa_s.put(256 * (7 * p + q) + r, 3 * j + m, w))

    def first_products(parts):
        for j, m in parts:
            if j == 0 or m == 0:
                landed()
            if (j, m) == (1, 0):
                queue_x(1)
            for k in {(0, 1): ((0, 1), (1, 0)), (0, 2): ((0, 2), (1, 1)), (1, 0): ((1, 2),)}.get((j, m), ()):
                queue_wa(*k, WA_GAP1 if j else WA_GAP0)
            for g in range(4 * j, 4 * j + 4):
                if (m, g) == (0, 2):
                    landed()
                    queue_wa(0, 0, WA_GAP00)
                rhs = w2_s[m * D:(m + 1) * D, 128 * g:128 * (g + 1)]
                lo = pacer.dot(xn_s.get(0, TB, 0, 4), rhs[:512], TB)
                yield
                c = lo + pacer.dot(xn_s.get(0, TB, 4, 8), rhs[512:], TB)
                if m == 0:
                    q_s.put(0, g, c * qscale)
                elif m == 1:
                    k_s.put(0, g, c)
                else:
                    vt_s.put(128 * g, 0, c.T)
                    pacer.due(c.T[120:128, TB - 128:], T_DELAY)
                yield

    count = [0, 0]

    def qkv_products(blk, j):
        for m in range(3):
            pacer.flush(("wa", j, m))
            if m == 0 and j == 0 and blk + 1 < NB:
                queue_x(blk + 1)
            low = {}
            for p in BAL1:
                order = BAL2[count[0] % 2]
                count[0] += 1
                prod = {}
                for q in order:
                    o = (blk % 2 * 49 + 7 * p + q) * QB
                    rhs = _halves(wa_s.get(256 * (7 * p + q), 256 * (7 * p + q + 1), 3 * j + m))
                    prod[q] = pacer.dot(xa_s.get(o, o + QB, 0, 2), rhs, QB, count[1] % 2)
                    count[1] += 1
                    if q == order[-1]:
                        low[p] = _bal_out(prod, order)
                        if p == BAL1[-1]:
                            finish_qkv(blk, j, m, low)
                    if count[1] % 2 == 0:
                        yield

    def finish_qkv(blk, j, m, low):
        c = {}
        for i in range(2):
            for k in range(2):
                t = _bal_out({p: low[p][i][k] for p in BAL1}, BAL1)
                c.update({(2 * hi + i, 2 * hj + k): t[hi][hj] for hi in range(2) for hj in range(2)})
        turn = ((0, 1), (0, 0), (1, 0), (1, 1))
        for hi, hj in turn:
            for i, k in turn:
                a, b = 2 * hi + i, 2 * hj + k
                v = c[a, b] * ((qscale if m == 0 else 1.0) / (12 * _ROW[a] * _COL[b]))
                if m == 0:
                    q_s.put(blk % 2 * TB + a * QB, 4 * j + b, v)
                elif m == 1:
                    k_s.put(blk * TB + a * QB, 4 * j + b, v)
                else:
                    v = v.T
                    vt_s.put(128 * (4 * j + b), 4 * blk + a, v)
        if m == 2:
            pacer.due(v[120:128], T_DELAY)

    def scores(sb, g, slot):
        j0 = max(0, 8 - 4 * sb)
        ss, ms = [], []
        b0, b1 = _lane_bits((16, 128))
        for t in range(4):
            qt = q_s.get(128 * (sb % 8) + 32 * t, 128 * (sb % 8) + 32 * (t + 1), g)
            q2 = [jnp.where(b0, qt, 0), jnp.where(b0, 0, qt)]
            q4 = [jnp.where(b1, q2[0], 0), jnp.where(b1, q2[1], 0), jnp.where(b1, 0, q2[0]), jnp.where(b1, 0, q2[1])]
            rhs = _halves(_cat([q4[c ^ t] for c in range(4)], 0))
            lo = max(j0, t)
            s = _dot_nt(_halves(k_s.get(128 * sb - W + 32 * lo, 128 * sb - W + 32 * (t + 9), g)), rhs)
            if t == 3:
                pacer.tick(s, s.shape[0])
            ch = {r: s[32 * (r + t - lo):32 * (r + t - lo + 1)] for r in range(lo - t, 9)}
            ch[8] = jnp.where(top_valid, ch.pop(0) if lo == t else -1e30, ch[8])
            m = None
            for r in sorted(ch):
                m = ch[r] if m is None else jnp.maximum(m, ch[r])
            ss.append(ch)
            ms.append(jnp.broadcast_to(jnp.max(m, axis=0, keepdims=True), (8, 128)))
        ls = [None] * 4
        words = {}

        def job(j, t):
            r = j - t
            p = jnp.exp2(ss[t][r or 8] - _cat([pacer.after(ms[t])] * 4, 0))
            l = (p[0:8] + p[8:16]) + (p[16:24] + p[24:32])
            ls[t] = l if ls[t] is None else ls[t] + l
            e_s[:, 128 * t:128 * (t + 1)] = _words(p)
            words[j, t] = e_s[:, 128 * t:128 * (t + 1)]
            if r == 0:
                words[j + 8, t] = words[j, t] & ~top_words
                words[j, t] = words[j, t] & top_words

        def emit(j):
            v = [words.get((j, t), jnp.zeros((16, 128), I32)) for t in range(4)]
            for h, w in enumerate(_butterfly(v)):
                p_s.put_words(384 * slot + 32 * j, h, w)

        for j in range(j0, 12):
            for t in range(4):
                if 0 <= j - t < 8 or (j - t == 8 and t < j0):
                    pacer.add("exp", EXP_GAP, lambda j=j, t=t: job(j, t), (sb, g))
            pacer.add("exp", 0, lambda j=j: emit(j), (sb, g))
        return ls

    def values(sb, g, slot, ls):
        j0 = max(0, 8 - 4 * sb)
        pacer.flush((sb, g))
        inv = _butterfly([pltpu.reciprocal(jnp.sum(l, axis=0, keepdims=True), full_range=False) for l in ls])
        outs = []
        for h in range(4):
            vt = _halves(vt_s.get(128 * g + DH * h, 128 * g + DH * (h + 1), sb - 2 + j0 // 4, sb + 1))
            ph = _halves(p_s.get(384 * slot + 32 * j0, 384 * (slot + 1), h))
            outs.append(_dot(vt, ph) * inv[h])
        ot = _cat(outs, 0).T
        pacer.due(ot[120:128], T_DELAY)
        r0, c0 = 256 * (sb % 2), 256 * (g // 2 % 2)
        pacer.flush(("o", r0, c0))
        a0, b0 = r0 + 128 * (sb % 4 // 2), c0 + 128 * (g % 2)
        o_s[a0:a0 + 128, b0:b0 + 128] = _cat(_butterfly([ot[32 * c:32 * (c + 1)] for c in range(4)]), 0)
        if sb % 4 >= 2 and g % 2:
            pacer.free["o"] = max(pacer.free.get("o", 0), pacer.now + T_DELAY + 50)
            for r in range(0, 128, 16):
                def job(r=r):
                    a = [[o_s[r0 + 128 * i + r:r0 + 128 * i + r + 16, c0 + 128 * b:c0 + 128 * (b + 1)]
                          for b in range(2)] for i in range(2)]
                    for i in range(2):
                        a[i][i] = _cat([pacer.after(a[i][i][:8]), a[i][i][8:]], 0)
                    for p, v in enumerate(_lhs7(a)):
                        oa_s.put(((sb // 4) * 7 + p) * HB + 128 * (sb % 2) + r, g // 2, v)
                pacer.add("o", O_GAP, job, ("o", r0, c0))

    def attention():
        units = [(4 * blk + s, 4 * j + (g ^ 2) + b) for blk in range(NB) for j in range(2) for g in (0, 2)
                 for s in (0, 2, 1, 3) for b in range(2)]
        units = units[max(0, 32 * BLK0 - 16):]
        prev = None
        for n, u in enumerate(units):
            ls = scores(*u, n % 3)
            yield
            if prev:
                values(*prev)
            prev = (*u, n % 3, ls)
            yield
        yield
        values(*prev)
        yield

    def queue_wo():
        for n in range(4):
            for r in range(0, 512, 16):
                def job(n=n, r=r):
                    t = {}
                    for a in range(2):
                        r0 = 128 * (2 * (r // 128) + a) + r % 128
                        w = wo_s[r0:r0 + 16, 256 * n:256 * (n + 1)].astype(F32)
                        for b in range(2):
                            v = w[:, 128 * b:128 * (b + 1)]
                            t[a, b] = _cat([pacer.after(v[:8]), v[8:]], 0) if a == b else v
                    for p in range(7):
                        wc_s.put(512 * p + r, n, _rhs7(p, lambda a, b: t[a, b]))
                pacer.add("w", WGT_GAP, job, "wo")

    def wo_products(blk):
        c = {}
        if blk == NB - 1:
            for slot in range(4):
                pacer.flush(("o", 256 * (slot // 2), 256 * (slot % 2)))
        for n in range(4):
            prod = {}
            for p in ORDER1:
                o = (blk * 7 + p) * HB
                prod[p] = pacer.dot(oa_s.get(o, o + HB, 0, 4), _halves(wc_s.get(512 * p, 512 * (p + 1), n)), HB)
                if p == ORDER1[-1]:
                    for i in range(2):
                        for b in range(2):
                            c[i, 2 * n + b] = _out4(prod.get, i, b, ORDER1)
                    if n == 3:
                        queue_h(blk, _cat([_cat([c[i, t] for t in range(8)], 1) for i in range(2)], 0))
                yield

    def queue_h(blk, o):
        hs = {}

        def normed(i, r):
            r0 = blk * TB + i * QB + r
            h = hs[i, r] = after_first(x_s[r0:r0 + 8, :].astype(F32)) + o[i * QB + r:i * QB + r + 8]
            if r % 16:
                x_s[r0 - 8:r0 + 8, :] = _cat([hs[i, r - 8], h], 0).astype(BF)
            return (yield from _ln(h if FUSE_LN else (yield from _ln(h)), (GS,)))
        queue_rows("h", blk, LNH_GAP if blk < NB - 1 else LNH_GAP_LAST, LNH_DELAY, LNH_GROUP, normed, (_lhs7,) + STD_TURN, ya_s,
                   lambda k: k * (S // 4) + blk * QB)

    def queue_w1(n, gap):
        for r in range(0, 256, 16):
            def tile(a, b, r=r):
                c0 = 512 * n + 256 * (b // 2)
                w = w1_s[256 * a + r:256 * a + r + 16, c0:c0 + 256].astype(F32)
                return w[:, 128 * (b % 2):128 * (b % 2 + 1)]
            queue_operands("w", gap, ("w1", n), lambda b: [_rhs7(p, lambda i, j: b[i][j]) for p in range(7)], *STD_TURN,
                           tile, lambda p, q, w, r=r: wb_s.put(256 * (7 * p + q) + r, n, w))

    def finish_early():
        x_s[0:16, 0:128] = _halves(pool[pl.ds(zero, 8), 0:128] | ya_pool[pl.ds(zero, 8), 0:128] | wb_pool[pl.ds(zero, 8), 0:128])
        cp = pltpu.make_async_copy(x_s, o_hbm, sem_out.at[0])
        cp.start()
        cp.wait()

    if PART & 1:
        ga = attention()
        if BLK0 == 0:
            for r in range(0, TB, 128):
                landed()

                def steps(r=r):
                    xn_s.put(r, 0, (yield from _ln(x_s[r:r + 128, :].astype(F32))))
                for _ in steps():
                    pass
            _interleave(first_products(((0, 0), (0, 1), (0, 2))), 24, ga, 0)
            _interleave(first_products(((1, 0), (1, 1), (1, 2))), 24, ga, ATT0)
        for blk in range(max(1, BLK0), NBT):
            finish_rows("x", blk)
            if blk == 1:
                landed()
                w2_copy.start()
            if blk == 2:
                landed()
                w2_copy.wait()
            if blk == 3:
                queue_wo()
                for n in W1_EARLY:
                    queue_w1(n, W1_GAP)
            split(f"b{blk}")
            for j in range(2):
                gp = qkv_products(blk, j)
                _interleave(gp, (147 + count[1] % 2) // 2, ga, 32 + (32 - ATT0 if (blk, j) == (1, 0) else 0))
                next(gp, None)
        if NBT < NB:
            landed()
            w2_copy.wait()
            return finish_early()
        pacer.flush("wo")
        _interleave(wo_products(0), 28, ga, 17)
        _interleave(wo_products(1), 28, ga, 17)
        for blk in range(2, NB):
            if blk == 2:
                split("w1")
            for _ in wo_products(blk):
                pass
    else:
        while stages:
            landed()
        w2_copy.start()
        w2_copy.wait()
        for n in W1_EARLY:
            queue_w1(n, 0)
            pacer.flush(("w1", n))
    if not PART & 2:
        finish_rows("h", NB - 1)
        return finish_early()

    b1 = b1_s[...].astype(F32).reshape(1, F) * GS
    b2 = b2_s[...].astype(F32).reshape(1, D)

    def queue_gelu(n, m1):
        bias = [jnp.broadcast_to(b1[:, 512 * n + 128 * b:512 * n + 128 * (b + 1)], (8, 128)) for b in range(4)]
        keys = [(i, j, hj) for i, j in ((0, 1), (1, 0), (0, 0), (1, 1)) for hj in range(2)]
        tied = {k: [] for k in keys}

        def finish():
            zs = []
            for i, j, hj in keys:
                m = {p: m1[p][i][j] for p in ORDER1}
                m[3 - hj] = m[3 - hj] + _cat(tied[i, j, hj], 0)
                zs += [_out4(m.get, hi, hj, [p for p in ORDER1 if p != 3 - hj] + [3 - hj]) for hi in range(2)]
            z = _cat([v[r:r + 16] for r in range(0, S // 4, 16) for v in zs], 0)
            g = z * jnp.tanh(z * (z * z + GK)) + z
            a = [[None] * 4 for _ in range(4)]
            for k, (i, j, hj) in enumerate(keys):
                for hi in range(2):
                    a[2 * hi + i][2 * hj + j] = _cat([g[16 * (r + 2 * k + hi):16 * (r + 2 * k + hi + 1)]
                                                      for r in range(0, S // 4, 16)], 0)
            for (p, q), v in _nested(_lhs7, a).items():
                ga_s.put(*ga_at(p, q, n), v)

        for r in range(0, S // 4, 16):
            for k in keys:
                def job(r=r, k=k):
                    tied[k] += [pacer.after(bias[2 * k[2] + k[1]])] * 2
                    if (r, k) == (S // 4 - 16, keys[-1]):
                        finish()
                pacer.add("g", GELU_GAP if n < NP - 1 else GELU_GAP_LAST, job)

    count[:] = [0, 0]
    for n in range(NPT):
        split(f"n{n}")
        pacer.flush(("w1", n))
        for k in W1_LATE[n]:
            queue_w1(k, 7800 / 112 / len(W1_LATE[n]))

        count[:] = [0, 0]

        def level2(p, b0, b1):
            order = ORDER2[count[0] % 2]
            count[0] += 1
            m = {}
            for q in order:
                d0 = (7 * p + q) * (S // 4)
                rhs = _halves(wb_s.get(256 * (7 * p + q), 256 * (7 * p + q + 1), n))
                r0, r1 = d0 + b0 * QB, d0 + b1 * QB
                if (p, q, b1) == (ORDER1[-1], order[-1], NB):
                    rm = (r0 + r1) // 2
                    m[q] = _cat([pacer.dot(ya_s.get(r0, rm, 0, 2), rhs, rm - r0, False),
                                 pacer.dot(ya_s.get(rm, r1, 0, 2), rhs, rm - r0)], 0)
                else:
                    m[q] = pacer.dot(ya_s.get(r0, r1, 0, 2), rhs, r1 - r0, count[1] % 2)
                count[1] += 1
            return m, order

        early = ORDER1[:NEARLY] if n == 0 else ()
        finish_rows("h", NB - 2)
        head = {p: level2(p, 0, NB - 1)[0] for p in early}
        finish_rows("h", NB - 1)
        pacer.dues = []
        if n == 0:
            for k in W1_TAIL:
                queue_w1(k, W1_GAP0)
        m1 = {}
        for p in ORDER1:
            if p in early:
                tail, order = level2(p, NB - 1, NB)
                m = {q: _cat([head[p][q], tail[q]], 0) for q in order}
            else:
                m, order = level2(p, 0, NB)
            m1[p] = [[_out4(m.get, i, j, order) for j in range(2)] for i in range(2)]
        queue_gelu(n, m1)

    if NPT < NP:
        pacer.flush("g")
        return finish_early()
    copies = []

    def send(win):
        cp = pltpu.make_async_copy(x_s.at[win], o_hbm.at[win], sem_out.at[len(copies)])
        cp.start()
        copies.append(cp)

    for n in range(2):
        split(f"m{n}")
        if n == 1:
            send((every, pl.ds(0, 512)))
        wt = w2_s[:, 512 * n:512 * (n + 1)].astype(F32)

        def level2(p, k0, k1):
            sub = _rhs_sub(lambda a, b: _cat([wt[512 * k + 128 * a:512 * k + 128 * (a + 1), 128 * b:128 * (b + 1)]
                                              for k in range(k0, k1)], 0), p)
            m = {}
            for q in ORDER1:
                d0, t0 = ga_at(p, q, 0)
                m[q] = pacer.dot(ga_s.get(d0, d0 + S // 4, t0 + k0, t0 + k1),
                                 _rhs7(q, lambda i, j: sub[i, j]).astype(BF), (k1 - k0) * S // 16)
            return m

        early = ORDER1[:KEARLY] if n == 0 else ()
        head = {p: level2(p, 0, NP - 1) for p in early}
        pacer.flush("g")
        if n == 0:
            split("w2")
        m1 = {}
        for p in ORDER1:
            if p in early:
                tail = level2(p, NP - 1, NP)
                m = {q: head[p][q] + tail[q] for q in ORDER1}
            else:
                m = level2(p, 0, NP)
            m1[p] = [[_out4(m.get, i, j, ORDER1) for j in range(2)] for i in range(2)]
            for hi in range(2):
                for hj in range(2):
                    if p != _last(hi, hj, ORDER1):
                        continue
                    c0 = 512 * n + 256 * hj
                    res = [_cat([_out4(lambda s: m1[s][i][j], hi, hj, ORDER1) for j in range(2)], 1) for i in range(2)]
                    for blk in range(NB):
                        win = (slice(blk * TB + 2 * QB * hi, blk * TB + 2 * QB * (hi + 1)), slice(c0, c0 + 256))
                        o = _cat([res[i][QB * blk:QB * (blk + 1)] for i in range(2)], 0)
                        x_s[win] = ((o * (0.5 / GS) + b2[:, c0:c0 + 256]) + x_s[win].astype(F32)).astype(BF)
            if n == 1 and p == ORDER1[-2]:
                send((every, pl.ds(768, 256)))
                for blk in range(NB):
                    send((pl.ds(blk * TB + 2 * QB, 2 * QB), pl.ds(512, 256)))
    for blk in range(NB):
        send((pl.ds(blk * TB, 2 * QB), pl.ds(512, 256)))
    for cp in copies:
        cp.wait()


@jax.jit
def pallas_sequential_preLN__sliding_block__mixer_channel_mlp__prompt_kernel(
        A_x, A_wqkv, A_wo, B_x, B_w1, B_b1, B_w2, B_b2):
    del B_x
    any_spec = pl.BlockSpec(memory_space=pl.ANY)
    out = pl.pallas_call(
        _kernel,
        out_shape=jax.ShapeDtypeStruct((S, D), BF),
        in_specs=[any_spec] * 7,
        out_specs=any_spec,
        scratch_shapes=[
            pltpu.VMEM((S, D), BF), pltpu.VMEM((D, D), BF), pltpu.VMEM((D, F), BF), pltpu.VMEM((F, D), BF),
            pltpu.VMEM((F,), BF), pltpu.VMEM((D,), BF),
            pltpu.VMEM((16, 512), I32), pltpu.VMEM((YSLOTS * 64, D), F32), pltpu.VMEM((512, 512), F32), pltpu.VMEM((3 * 384, 256), I32), pltpu.VMEM((49 * S // 8, 256), I32),
            pltpu.VMEM((49 * 128 * 4, 256), I32), pltpu.VMEM((46080, 256), I32),
            pltpu.SemaphoreType.DMA((18,)), pltpu.SemaphoreType.DMA((2 + 2 * NB,)),
        ],
        compiler_params=pltpu.CompilerParams(vmem_limit_bytes=127 << 20),
        name="fused_block",
    )(A_x.reshape(S, D), A_wqkv, A_wo, B_w1, B_b1, B_w2, B_b2)
    return out.reshape(1, S, D)
```

```python
import math

import jax
import jax.numpy as jnp
from jax import lax
import jax.experimental.pallas as pl
import jax.experimental.pallas.tpu as pltpu

S, D, F = 2048, 1024, 3584
DH, W = 32, 256
EPS = 1e-5
TB = 512
NB = S // TB
HB, QB = TB // 2, TB // 4
NP = F // 512
BF, F32, I32 = jnp.bfloat16, jnp.float32, jnp.int32

GS = (math.sqrt(2.0 / math.pi) * 0.044715) ** (1.0 / 3.0)
GK = math.sqrt(2.0 / math.pi) / GS

GAP = {
    "exp": 25, "o": 150, "x": (None, 116, 400, 400), "h": (130, 113, 113, 113),
    "wa": {(0, 0): 27, (0, 1): 36, (0, 2): 18, (1, 0): 18, (1, 1): 83, (1, 2): 135},
    "wo": 150, "w1": (100, 45, 45, 19, 19, 108, 108), "w2": (66, 66, 69.5) + (60.5,) * 4,
    "gelu": (48,) * (NP - 1) + (41.5,), "halves": 32, "finish": 150, "finish_last": 24,
}
COST = {"exp": 9, "o": 9, "xc": 9, "hc": 1, "w": 9, "g": 14, "a": 7, "f": 9}
COST_FIRST = {"xc": 24, "hc": 1, "w": 24}
W1_WHEN = {"qkv": (0,), "wo": (1, 2), 0: (3, 4), 1: (5,), 2: (6,)}
ROWS = 64
TRANSPOSE_TIME = 900
REDUCE_TIME = 180
NORM_TIME = 200
SCORE_PACE = 0.8
EARLY = ((2, 4), (3, 6))


def _cat(xs, axis):
    return xs[0] if len(xs) == 1 else lax.concatenate(xs, axis)


def _rows(x, r0, r1):
    return lax.slice_in_dim(x, r0, r1, axis=0)


def _tile(x, t, n=1):
    return lax.slice_in_dim(x, 128 * t, 128 * (t + n), axis=1)


def _words(x):
    return pltpu.bitcast(x.astype(BF), I32)


def _halves(w):
    return pltpu.bitcast(w, BF) if w.dtype == I32 else w


def _dot(a, b):
    return lax.dot_general(_halves(a), _halves(b), (((1,), (0,)), ((), ())), preferred_element_type=F32)


def _dot_nt(a, b):
    return lax.dot_general(_halves(a), _halves(b), (((1,), (1,)), ((), ())), preferred_element_type=F32)


def _layernorm(x, scales=None):
    m = jnp.mean(x, axis=-1, keepdims=True)
    yield
    xc = x - m
    v = jnp.mean(xc * xc, axis=-1, keepdims=True)
    yield
    r = lax.rsqrt(v + EPS)
    if scales is None:
        return xc * r
    n = x.shape[1] // 128 // len(scales)
    rs = {c: r * c for c in scales}
    return _cat([_tile(xc, n * i, n) * rs[c] for i, c in enumerate(scales)], 1)


def _lhs7(a):
    (a11, a12), (a21, a22) = a
    return [a11 + a22, a21 + a22, a11, a22, a11 + a12, a21 - a11, a12 - a22]


def _rhs7(b):
    (b11, b12), (b21, b22) = b
    return [b11 + b22, b11, b12 - b22, b21 - b11, b22, b11 + b12, b21 + b22]


_TERMS = {(0, 0): {0: 1, 3: 1, 4: -1, 6: 1}, (0, 1): {2: 1, 4: 1},
          (1, 0): {1: 1, 3: 1}, (1, 1): {0: 1, 1: -1, 2: 1, 5: 1}}
ORDER1 = (1, 3, 2, 4, 5, 0, 6)
ORDER2 = (ORDER1, (6, 1, 3, 2, 4, 5, 0))


def _out4(m, i, j, order):
    acc = None
    for p in reversed(order):
        sign = _TERMS[i, j].get(p)
        if sign and acc is None:
            acc = m(p) if sign > 0 else -m(p)
        elif sign:
            acc = acc + m(p) if sign > 0 else acc - m(p)
    return acc


def _last(i, j):
    return [p for p in ORDER1 if p in _TERMS[i, j]][-1]


_ROW = (1.0, math.sqrt(3.0), math.sqrt(3.0), 3.0)
_COL = _ROW[::-1]
BAL1 = (0, 1, 2, 4, 6, 3, 5)
BAL2 = ((1, 2, 4, 6, 3, 5, 0), BAL1)


def _bal_lhs7(a):
    (a11, a12), (a21, a22) = a
    s, t = a11 + a22, a12 + a21
    return [s, a11 - a12, a11 + a12, s - t, a12 - a22, s + t, a12 + a22]


def _bal_rhs7(b):
    (b11, b12), (b21, b22) = b
    s, t = b11 + b22, b12 + b21
    return [s + s, b12 - b22, b12 + b22, b11 + b12, s + t, b11 - b12, s - t]


def _bal_out(m, order):
    c12, e = m[1] + m[2], m[1] - m[2]
    c21 = (c12 - (m[4] + m[6])) + (m[5] - m[3])
    if order[0] == 0:
        d = e + m[0]
        return [[d + (m[4] - m[6]), c12], [c21, d - (m[3] + m[5])]]
    return [[(e + (m[4] - m[6])) + m[0], c12], [c21, (e - (m[3] + m[5])) + m[0]]]


STD_TURN = (ORDER1, ((0, 0), (1, 1)))
BAL_TURN = ((1, 2, 3, 5, 0, 4, 6), ((0, 0), (0, 1)))


def _nested(f, a, hold=lambda q, k, v: v):
    low = {(hi, hj): f([[a[2 * hi + i][2 * hj + j] for j in range(2)] for i in range(2)])
           for hi in range(2) for hj in range(2)}
    return {(p, q): v for q in range(7)
            for p, v in enumerate(f([[hold(q, (hi, hj), low[hi, hj][q]) for hj in range(2)] for hi in range(2)]))}


def _lane_bits(shape):
    lane = lax.broadcasted_iota(I32, shape, 1)
    return (lane & 32) == 0, (lane & 64) == 0


def _butterfly(v, b0, b1):
    u = [lax.select(b0, v[i], v[i ^ 1]) for i in range(4)]
    return [lax.select(b1, u[i], u[i ^ 2]) for i in range(4)]


class _Pacer:
    def __init__(self):
        self.masks = {}
        self.now = 0.0
        self.mark = None
        self.busy = 0.0
        self.free = {}
        self.events = []
        self.dues = []

    def tie(self, value, marks):
        known = [m for m in marks if m is not None]
        if not known:
            return value
        if value.shape not in self.masks:
            lane = lax.broadcasted_iota(I32, value.shape, 1) & 127
            self.masks[value.shape] = lane * lane == 2
        n = value.shape[0] // 8 // len(marks)
        wait = _cat([known[-1] if m is None else m for m in marks for _ in range(n)], 0)
        if wait.dtype != value.dtype:
            wait = pltpu.bitcast(wait, value.dtype)
        return lax.select(self.masks[value.shape], _cat([wait] * (value.shape[1] // 128), 1), value)

    def due(self, value, delay):
        self.dues.append((self.now + delay, pltpu.bitcast(value, I32)))

    def at(self, t, tag, job):
        self.events.append((t, tag, job))
        self.events.sort(key=lambda e: e[0])

    def add(self, lane, gap, tag, job, delay=0):
        t = max(self.now + delay, self.free.get(lane, 0.0))
        self.free[lane] = t + gap
        self.at(t, tag, job)

    def collect(self, lane, gap, tag, n, then, delay=0, group=0):
        marks = []

        def job():
            marks.append(self.mark)
            if len(marks) == n:
                then(marks)
            return COST_FIRST[lane] if group and len(marks) % group == 1 else COST[lane]
        for _ in range(n):
            self.add(lane, gap, tag, job, delay)

    def stepwise(self, tag, steps):
        def job():
            if next(steps, self) is not self:
                self.at(self.now + REDUCE_TIME, tag, job)
            return 1
        return job

    def tick(self, r, cycles):
        n = r.shape[0] // 8
        for i in range(n):
            self.now += cycles / n
            if self.events and max(self.busy, self.events[0][0]) <= self.now:
                self.mark = lax.slice(r, (8 * i, 0), (8 * i + 8, 128))
                self.busy = self.now + self.events.pop(0)[2]()
        self.mark = None

    def flush(self, tag):
        while tag in [e[1] for e in self.events]:
            t, _, job = self.events.pop([e[1] for e in self.events].index(tag))
            self.now, now = t, self.now
            job()
            self.now = now

    def dot(self, lhs, rhs, cycles, last=True):
        n = lhs.shape[0]
        for t, v in self.dues:
            if t < self.now + cycles:
                i = 8 * max(0, int((t - self.now) * (n // 8) / cycles))
                parts = [_rows(lhs, 0, i)] if i else []
                parts.append(self.tie(_rows(lhs, i, i + 8), [v]))
                lhs = _cat(parts + ([_rows(lhs, i + 8, n)] if i + 8 < n else []), 0)
        r = _dot(lhs, rhs)
        if last:
            self.dues = [d for d in self.dues if d[0] >= self.now + cycles]
            self.tick(r, cycles)
        return r


class _Words:
    def __init__(self, pool, start, rows, tiles):
        self.pool, self.start, self.rows = pool, start, rows // 2
        self.end = start + self.rows * ((tiles + 1) // 2)
        assert self.end <= pool.shape[0]

    def _window(self, r0, n, t, k):
        r = self.start + (t // 2) * self.rows + r0 // 2
        return slice(r, r + n), slice(128 * (t % 2), 128 * (t % 2 + k))

    def _runs(self, t0, t1):
        while t0 < t1:
            k = 2 if t0 % 2 == 0 and t0 + 1 < t1 else 1
            yield t0, k
            t0 += k

    def get(self, r0, r1, t0, t1=None):
        return _cat([self.pool[self._window(r0, (r1 - r0) // 2, t, k)] for t, k in self._runs(t0, t1 or t0 + 1)], 1)

    def put(self, r0, t0, x):
        runs = list(self._runs(t0, t0 + x.shape[1] // 128))
        for t, k in runs:
            part = x if len(runs) == 1 else _tile(x, t - t0, k)
            self.pool[self._window(r0, x.shape[0] // 2, t, k)] = _words(part)


def _interleave(a, na, b, nb):
    ia = ib = 0
    while ia < na or ib < nb:
        if ib >= nb or (ia < na and ia * nb <= ib * na):
            next(a)
            ia += 1
        else:
            next(b)
            ib += 1


def _kernel(x_hbm, wqkv_hbm, wo_hbm, w1_hbm, b1_hbm, w2_hbm, b2_hbm, o_hbm,
            x_s, wo_s, w1_s, w2_s, b1_s, b2_s, y_s, o_s, p_pool, ya_pool, wb_pool, pool, sem_in, sem_out):
    pacer = _Pacer()
    sems = iter(range(sem_in.shape[0]))

    def copy(src, dst):
        return pltpu.make_async_copy(src, dst, sem_in.at[next(sems)])

    def wqkv_copy(m, c0, n):
        return copy(wqkv_hbm.at[:, pl.ds(m * D + c0, n)], w2_s.at[pl.ds(m * D, D), pl.ds(c0, n)])

    def row_copy(src, dst, r0, r1):
        return copy(src.at[pl.ds(r0, r1 - r0)], dst.at[pl.ds(r0, r1 - r0)])

    stages = [[row_copy(x_hbm, x_s, r, r + QB)] for r in range(0, TB, QB)] + [
        [wqkv_copy(0, 0, 128)],
        [wqkv_copy(0, 128, 384)],
        [wqkv_copy(1, 0, 512)],
        [wqkv_copy(2, 0, 512), wqkv_copy(0, 512, 512)],
        [wqkv_copy(1, 512, 512), wqkv_copy(2, 512, 512), row_copy(x_hbm, x_s, TB, 2 * TB)],
    ]
    rest = [row_copy(x_hbm, x_s, 2 * TB, S), copy(b1_hbm, b1_s), copy(b2_hbm, b2_s), copy(wo_hbm, wo_s)]
    w1_copy = copy(w1_hbm, w1_s)
    w2_copies = [row_copy(w2_hbm, w2_s, r, r + F // 2) for r in (0, F // 2)]
    for stage in stages + [rest]:
        for c in stage:
            c.start()

    def landed():
        for c in stages.pop(0):
            c.wait()

    lane = lax.broadcasted_iota(I32, (32, 128), 1)
    row = lax.broadcasted_iota(I32, (32, 128), 0)
    top_valid = row > (lane & 31)
    lane16 = lax.broadcasted_iota(I32, (16, 128), 1)
    row16 = lax.broadcasted_iota(I32, (16, 128), 0)
    top_words = (jnp.where(2 * row16 > (lane16 & 31), 0xFFFF, 0)
                 | jnp.where(2 * row16 + 1 > (lane16 & 31), -0x10000, 0))
    low_words = ~top_words

    zero = jnp.clip((lane16 * lane16)[0, 0], 0, 1) * 8
    for buf in (y_s, o_s, p_pool, ya_pool, wb_pool, pool):
        buf[pl.ds(zero, 8), 0:128] = jnp.zeros((8, 128), buf.dtype)
    p_s = _Words(p_pool, 0, 3 * W, 4)
    xa_s = _Words(pool, 0, 2 * 49 * QB, 2)
    oa_s = _Words(pool, xa_s.end, 7 * S // 2, 4)
    q_s = _Words(pool, oa_s.end, 2 * TB, 8)
    k_s = _Words(pool, q_s.end, S, 8)
    vt_s = _Words(pool, k_s.end, D, S // 128)
    wa_s = _Words(pool, vt_s.end, 49 * 256, 6)
    xn_s = _Words(pool, wa_s.end, TB, 8)
    wc_s = _Words(pool, wa_s.end, 7 * 512, 4)
    ya_s = _Words(ya_pool, 0, 49 * S // 4, 2)
    wb_s = _Words(wb_pool, 0, 49 * 256, NP)
    ga_s = _Words(pool, 0, 25 * S // 4, 2 * NP)
    gc_s = _Words(pool, ga_s.end, 14 * HB, 3)
    we_s = _Words(wb_pool, 0, 49 * 128, 2)
    wd_s = _Words(wb_pool, we_s.end, 21 * 4 * 384, 2)

    def split(wait=(), start=()):
        for c in wait:
            c.wait()
        for c in start:
            c.start()

        @pl.when(zero != 0)
        def _():
            pool[0:8, 0:128] = jnp.zeros((8, 128), I32)

    def x_rows(r0):
        x = x_s[r0:r0 + 8, :].astype(F32)
        return _cat([pacer.tie(_tile(x, 0), [pacer.mark]), _tile(x, 1, 7)], 1)

    def queue_operands(lane, gap, tag, steps, combine, turn, block, put, delay=0):
        order, held = turn

        def emit(marks):
            def hold(q, k, v):
                return pacer.tie(v, marks[order.index(q)::7]) if k in held else v
            for (p, q), v in _nested(combine, [[block(a, b) for b in range(4)] for a in range(4)], hold).items():
                put(7 * p + q, v)
        pacer.collect(lane, gap, tag, 7 * steps, emit, delay, 7)

    def queue_rows(lane, blk, group, normed, combine, turn, dest, row0):
        gap = GAP[lane][blk]
        done = []

        def steps(i, r):
            y = yield from normed(i, r)
            r0 = r // 16 * 16
            y0 = TB * (blk % 2) + r0
            y_s[y0 + QB * i + r - r0:y0 + QB * i + r - r0 + 8, :] = y
            done.append(_tile(y, 0))
            if len(done) % group == 0:
                pacer.due(sum(done[1 - group:], done[-group]), NORM_TIME)
            if len(done) % 8 == 0:
                for c in range(2):
                    queue_operands(
                        lane + "c", gap * 8 / 15, (lane, blk), 1, combine, turn,
                        lambda a, b, c=c: y_s[y0 + QB * a:y0 + QB * a + 16, 256 * b + 128 * c:256 * b + 128 * (c + 1)],
                        lambda k, v, c=c: dest.put(row0(k) + r0, c, v), NORM_TIME + 50)
        pacer.flush((lane, blk - 2))
        for r in range(0, QB, 16):
            for i in range(4):
                for rr in (r, r + 8):
                    pacer.add(lane, gap, (lane, blk), pacer.stepwise((lane, blk), steps(i, rr)))

    qscale = (DH ** -0.5) * math.log2(math.e)
    count = [0, 0]
    bits = {n: _lane_bits((n, 128)) for n in (1, 16, 32, 64, 128, 192)}
    nought = jnp.zeros((16, 128), I32)

    def queue_x(blk):
        queue_rows("x", blk, 2 if blk > 1 else 4,
                   lambda i, r: _layernorm(x_rows(blk * TB + i * QB + r), [_ROW[i] * c for c in _COL]),
                   _bal_lhs7, BAL_TURN, xa_s, lambda k: (blk % 2 * 49 + k) * QB)

    def queue_wa(j, m):
        def block(a, b):
            r0, c0 = m * D + 256 * a, 512 * j + 256 * (b // 2)
            return _tile(w2_s[r0:r0 + 256, c0:c0 + 256].astype(F32), b % 2) * (_ROW[a] * _COL[b])
        queue_operands("w", GAP["wa"][j, m], ("wa", j, m), 16, _bal_rhs7, BAL_TURN, block,
                       lambda k, v: wa_s.put(256 * k, 3 * j + m, v))

    def put_qkv(m, r0, g, c):
        if m == 0:
            q_s.put(r0 % (2 * TB), g, c)
        elif m == 1:
            k_s.put(r0, g, c)
        else:
            c = c.T
            vt_s.put(128 * g, r0 // 128, c)
        return lax.slice(c, (c.shape[0] - 8, c.shape[1] - 128), c.shape)

    def first_products(j, m):
        for g in range(4 * j, 4 * j + 4):
            if (m, g) == (0, 1):
                landed()
                queue_wa(0, 0)
            c = pacer.dot(xn_s.get(0, TB, 0, 4), w2_s[m * D:m * D + 512, 128 * g:128 * (g + 1)], TB)
            yield
            c += pacer.dot(xn_s.get(0, TB, 4, 8), w2_s[m * D + 512:(m + 1) * D, 128 * g:128 * (g + 1)], TB)
            last = put_qkv(m, 0, g, c * qscale if m == 0 else c)
            if m == 2:
                pacer.due(last, TRANSPOSE_TIME)
            yield

    def qkv_products(blk, j):
        for m in range(3):
            pacer.flush(("wa", j, m))
            low = {}
            for p in BAL1:
                order = BAL2[count[0] % 2]
                count[0] += 1
                prod = {}
                for q in order:
                    k = 7 * p + q
                    o = (blk % 2 * 49 + k) * QB
                    prod[q] = pacer.dot(xa_s.get(o, o + QB, 0, 2), wa_s.get(256 * k, 256 * (k + 1), 3 * j + m),
                                        QB * (876 - 288 * SCORE_PACE) / 588, count[1] % 2)
                    count[1] += 1
                    if q == order[-1]:
                        low[p] = _bal_out(prod, order)
                        if p == BAL1[-1]:
                            finish_qkv(blk, j, m, low)
                    if count[1] % 2 == 0:
                        yield

    def finish_qkv(blk, j, m, low):
        c = {}
        for i in range(2):
            for k in range(2):
                t = _bal_out({p: low[p][i][k] for p in BAL1}, BAL1)
                c.update({(2 * hi + i, 2 * hj + k): t[hi][hj] for hi in range(2) for hj in range(2)})
        turn = ((0, 1), (0, 0), (1, 0), (1, 1))
        for hi, hj in turn:
            for i, k in turn:
                a, b = 2 * hi + i, 2 * hj + k
                scale = (qscale if m == 0 else 1.0) / (12 * _ROW[a] * _COL[b])
                last = put_qkv(m, blk * TB + a * QB, 4 * j + b, c[a, b] * scale)
        if m == 2:
            pacer.due(last, TRANSPOSE_TIME)

    def scores(sb, g, slot, turn=(0, 1, 2, 3)):
        j0 = max(0, 8 - 4 * sb)
        ss, ms = {}, {}
        b0, b1 = bits[16]
        for t in turn:
            qt = q_s.get(128 * (sb % 8) + 32 * t, 128 * (sb % 8) + 32 * (t + 1), g)
            q2 = [lax.select(b0, qt, nought), lax.select(b0, nought, qt)]
            q4 = [lax.select(b1, v, nought) for v in q2] + [lax.select(b1, nought, v) for v in q2]
            lo = max(j0, t)
            keys = k_s.get(128 * sb - W + 32 * lo, 128 * sb - W + 32 * (t + 9), g)
            s = _dot_nt(keys, _cat([q4[c ^ t] for c in range(4)], 0))
            n = s.shape[0]
            if t == 3:
                pacer.tick(s, n * SCORE_PACE)
            first = _rows(s, 0, 32) if lo == t else jnp.full((32, 128), -jnp.inf, F32)
            body = [_rows(s, 32 if lo == t else 0, n - 32)] if n > 32 else []
            ss[t] = _cat(body + [lax.select(top_valid, first, _rows(s, n - 32, n))], 0)
            ms[t] = jnp.broadcast_to(jnp.max(ss[t], axis=0, keepdims=True), (8, 128))
        todo = [(j, t) for j in range(j0, 12) for t in range(4) if 0 <= j - t < 8 or (j - t == 8 and t < j0)]
        sums = []

        def emit(marks):
            ends = [ss[t].shape[0] - (0 if j == t else 32 * (8 + t - j)) for j, t in todo]
            s = _cat([_rows(ss[t], e - 32, e) for (_, t), e in zip(todo, ends)], 0)
            p = jnp.exp2(s - pacer.tie(_cat([ms[t] for _, t in todo for _ in range(4)], 0), marks))
            for t in range(4):
                pt = _cat([_rows(p, 32 * k, 32 * (k + 1)) for k, (_, u) in enumerate(todo) if u == t], 0)
                sums.append(jnp.sum(pt, axis=0, keepdims=True))
                p_s.put(W * slot, t, pt)
        pacer.collect("exp", GAP["exp"], (sb, g), len(todo), emit)
        return sums

    def values(sb, g, slot, sums):
        j0 = max(0, 8 - 4 * sb)
        pacer.flush((sb, g))
        inv = _butterfly([pltpu.reciprocal(l, full_range=False) for l in sums], *bits[1])
        v = []
        for t in range(4):
            n = min(8, 9 + t - j0)
            w = p_s.get(W * slot, W * slot + 32 * n, t)
            parts = [w]
            if t >= j0:
                edge = _rows(w, 0, 16)
                parts = [nought] * (t - j0) + [edge & top_words, _rows(w, 16, 16 * n), edge & low_words]
            v.append(_cat(parts + [nought] * (3 - t), 0))
        heads = _butterfly(v, *bits[v[0].shape[0]])
        outs = [None] * 4
        for k in range(3 - j0 // 4):
            for h in range(4):
                vt = vt_s.get(128 * g + DH * h, 128 * g + DH * (h + 1), sb - 2 + j0 // 4 + k)
                o = _dot(vt, _rows(heads[h], 64 * k, 64 * (k + 1)))
                outs[h] = o if k == 0 else outs[h] + o
        ot = _cat([o * i for o, i in zip(outs, inv)], 0).T
        pacer.due(_rows(ot, 120, 128), TRANSPOSE_TIME)
        r0, c0 = 256 * (sb % 2), 256 * (g // 2 % 2)
        pacer.flush(("o", r0, c0))
        a0, b0 = r0 + 128 * (sb % 4 // 2), c0 + 128 * (g % 2)
        o_s[a0:a0 + 128, b0:b0 + 128] = _cat(_butterfly([_rows(ot, r, r + 32) for r in range(0, 128, 32)], *bits[32]), 0)
        if sb % 4 >= 2 and g % 2:
            def emit(marks):
                a = [[o_s[r0 + 128 * i:r0 + 128 * (i + 1), c0 + 128 * b:c0 + 128 * (b + 1)] for b in range(2)]
                     for i in range(2)]
                for i in range(2):
                    a[i][i] = pacer.tie(a[i][i], marks)
                for p, v in enumerate(_lhs7(a)):
                    oa_s.put(((sb // 4) * 7 + p) * HB + 128 * (sb % 2), g // 2, v)
            pacer.collect("o", GAP["o"], ("o", r0, c0), 8, emit, TRANSPOSE_TIME + 50)

    def attention():
        units = [(4 * blk + s, 4 * j + g + b) for blk in range(NB) for j in range(2) for g in (2, 0)
                 for s in (0, 2, 1, 3) for b in range(2)]
        prev = None
        for n, u in enumerate(units):
            if u[0] >= 2:
                sums = scores(*u, n % 3)
            elif n % 2 == 0:
                sums = scores(*u, n % 3)
                ahead = scores(*units[n + 1], (n + 1) % 3, (3, 2, 1, 0))
            else:
                sums = ahead
            yield
            if prev:
                values(*prev)
            prev = (*u, n % 3, sums)
            yield
        yield
        values(*prev)
        yield

    def queue_wo(n):
        def emit(marks):
            def block(a, b):
                w = _cat([wo_s[128 * k:128 * (k + 1), 256 * n:256 * (n + 1)] for k in range(a, 8, 2)], 0)
                w = _tile(w.astype(F32), b)
                return pacer.tie(w, marks) if a == b else w
            for p, v in enumerate(_rhs7([[block(a, b) for b in range(2)] for a in range(2)])):
                wc_s.put(512 * p, n, v)
        pacer.collect("w", GAP["wo"], "wo", 32, emit)

    def wo_products(blk):
        c = {}
        for n in range(4):
            prod = {}
            for p in ORDER1:
                o = (blk * 7 + p) * HB
                prod[p] = pacer.dot(oa_s.get(o, o + HB, 0, 4), wc_s.get(512 * p, 512 * (p + 1), n), HB)
                if p == ORDER1[-1]:
                    for i in range(2):
                        for b in range(2):
                            c[i, 2 * n + b] = _out4(prod.get, i, b, ORDER1)
                    if n == 3:
                        queue_h(blk, _cat([_cat([c[i, t] for t in range(8)], 1) for i in range(2)], 0))
                yield

    def queue_h(blk, o):
        hs = {}

        def normed(i, r):
            r0 = blk * TB + i * QB + r
            h = hs[i, r] = x_rows(r0) + _rows(o, i * QB + r, i * QB + r + 8)
            if r % 16:
                x_s[r0 - 8:r0 + 8, :] = _cat([hs[i, r - 8], h], 0).astype(BF)
            return (yield from _layernorm((yield from _layernorm(h)), (GS,)))
        queue_rows("h", blk, 4, normed, _lhs7, STD_TURN, ya_s, lambda k: k * (S // 4) + blk * QB)

    def queue_w1(n):
        def block(a, b):
            c0 = 512 * n + 256 * (b // 2)
            return _tile(w1_s[256 * a:256 * (a + 1), c0:c0 + 256].astype(F32), b % 2)
        queue_operands("w", GAP["w1"][n], ("w1", n), 16, _rhs7, STD_TURN, block,
                       lambda k, v: wb_s.put(256 * k, n, v))

    ga = attention()
    for r in range(0, TB, QB):
        landed()

        def steps(r=r):
            xn_s.put(r, 0, (yield from _layernorm(x_s[r:r + QB, :].astype(F32))))
        list(steps())
    landed()
    list(first_products(0, 0))
    landed()
    queue_wa(0, 1)
    list(first_products(0, 1))
    landed()
    queue_wa(0, 2)
    queue_wa(1, 0)
    list(first_products(0, 2))
    _interleave(first_products(1, 0), 8, ga, 17)
    landed()
    queue_x(1)
    queue_wa(1, 1)
    _interleave((None for m in (1, 2) for _ in first_products(1, m)), 16, ga, 14)
    for blk in range(1, NB):
        pacer.flush(("x", blk))
        if blk == 1:
            queue_wa(1, 2)
            split(wait=rest, start=[w1_copy])
        if blk < NB - 1:
            queue_x(blk + 1)
        else:
            split(wait=[w1_copy])
            for n in range(4):
                queue_wo(n)
            for n in W1_WHEN["qkv"]:
                queue_w1(n)
        for j in range(2):
            gp = qkv_products(blk, j)
            _interleave(gp, (147 + count[1] % 2) // 2, ga, 32)
            next(gp, None)
    pacer.flush("wo")
    for n in W1_WHEN["wo"]:
        queue_w1(n)
    _interleave(wo_products(0), 28, ga, 17)
    _interleave(wo_products(1), 28, ga, 18)
    split(start=w2_copies[:1])
    list(wo_products(2))
    for r0 in (0, 256):
        for c0 in (0, 256):
            pacer.flush(("o", r0, c0))
    list(wo_products(3))

    b1 = b1_s[...].astype(F32).reshape(1, F) * GS
    b2 = b2_s[...].astype(F32).reshape(1, D)

    def ga_at(p, q):
        k = 7 * p + q
        return k // 2 * (S // 4), k % 2 * NP

    def queue_gelu(n, low):
        keys = [(i, j, hj) for i, j in ((0, 1), (1, 0), (0, 0), (1, 1)) for hj in range(2)]

        def emit(marks):
            zs = []
            for k, (i, j, hj) in enumerate(keys):
                m = {p: low[p][i][j] for p in ORDER1}
                both = 3 - hj
                bias = jnp.broadcast_to(_tile(b1, 4 * n + 2 * hj + j), (S // 4, 128))
                m[both] = m[both] + pacer.tie(bias, marks[k::8])
                zs += [_out4(m.get, hi, hj, [p for p in ORDER1 if p != both] + [both]) for hi in range(2)]
            z = _cat([_rows(v, r, r + 16) for r in range(0, S // 4, 16) for v in zs], 0)
            g = z * jnp.tanh(z * (z * z + GK)) + z
            a = [[None] * 4 for _ in range(4)]
            for k, (i, j, hj) in enumerate(keys):
                for hi in range(2):
                    a[2 * hi + i][2 * hj + j] = _cat([_rows(g, 16 * (r + 2 * k + hi), 16 * (r + 2 * k + hi + 1))
                                                      for r in range(0, S // 4, 16)], 0)
            for (p, q), v in _nested(_lhs7, a).items():
                d0, t0 = ga_at(p, q)
                ga_s.put(d0, t0 + n, v)
        pacer.collect("g", GAP["gelu"][n], ("g", n), 8 * S // 64, emit)

    def queue_w2(k):
        p = ORDER1[k]

        def inner(positions, n):
            def block(a, b):
                c0 = 512 * n + 256 * (b // 2)
                w = [w2_s[512 * t + 128 * a:512 * t + 128 * (a + 1), c0:c0 + 256].astype(F32) for t in positions]
                return _tile(_cat(w, 0), b % 2)
            return _rhs7([[_rhs7([[block(2 * hi + i, 2 * hj + j) for hj in range(2)] for hi in range(2)])[p]
                           for j in range(2)] for i in range(2)])

        def emit(marks):
            low = [[inner(range(3 * i, 3 * i + 3), n) for n in range(2)] for i in range(2)]
            for q in range(7):
                v = [[low[i][n][q] for n in range(2)] for i in range(2)]
                for i in range(2):
                    for n in (i,) if k else range(2):
                        v[i][n] = pacer.tie(v[i][n], marks[ORDER1.index(q)::7])
                for r, w in enumerate(_rhs7(v) if k else v[0] + v[1]):
                    wd_s.put(384 * (4 * (7 * (k % 3) + q) + r // 2), r % 2, w)

        def emit_seventh(marks):
            for n in range(2):
                for q, w in enumerate(inner([NP - 1], n)):
                    we_s.put(128 * (7 * p + q), n, pacer.tie(w, marks[n::2]))
        pacer.collect("w", GAP["w2"][k], ("w2", k), 16, emit_seventh)
        pacer.collect("w", GAP["w2"][k], ("w2", k), 7 * 24, emit, 0, 7)

    def w1_products(n, p, b0, b1):
        order = ORDER2[count[0] % 2]
        count[0] += 1
        m = {}
        for q in order:
            k = 7 * p + q
            rhs = wb_s.get(256 * k, 256 * (k + 1), n)
            r0, r1 = k * (S // 4) + b0 * QB, k * (S // 4) + b1 * QB
            if (p, q, b1) == (ORDER1[-1], order[-1], NB):
                rm = (r0 + r1) // 2
                m[q] = _cat([pacer.dot(ya_s.get(r0, rm, 0, 2), rhs, rm - r0, False),
                             pacer.dot(ya_s.get(rm, r1, 0, 2), rhs, rm - r0)], 0)
            else:
                m[q] = pacer.dot(ya_s.get(r0, r1, 0, 2), rhs, r1 - r0, count[1] % 2)
            count[1] += 1
        return m, order

    low = None
    for n in range(NP):
        pacer.flush(("w1", n))
        if n in (1, 5):
            pacer.flush(("g", n - 2))
            split(wait=w2_copies if n == 5 else (), start=w2_copies[1:] if n == 1 else ())
        if n:
            queue_gelu(n - 1, low)
        if n >= NP - 2:
            queue_w2(n - NP + 2)
        count[:] = [0, 0]
        done = {p: (0, []) for p in ORDER1}
        if n == 0:
            for upto, some in EARLY:
                for b in range(upto):
                    pacer.flush(("h", b))
                for p in ORDER1[:some]:
                    done[p] = (upto, done[p][1] + [w1_products(n, p, done[p][0], upto)[0]])
            pacer.flush(("h", NB - 1))
            pacer.dues = []
        for k in W1_WHEN.get(n, ()):
            queue_w1(k)
        low = {}
        for p in ORDER1:
            tail, order = w1_products(n, p, done[p][0], NB)
            m = {q: _cat([v[q] for v in done[p][1] + [tail]], 0) for q in order}
            low[p] = [[_out4(m.get, i, j, order) for j in range(2)] for i in range(2)]
    for n in range(NP - 1):
        pacer.flush(("g", n))
    queue_gelu(NP - 1, low)

    turn = [(p, q) for p in ORDER1 for q in ORDER1]
    scale = 0.5 / GS
    low, partial, copies = {}, {}, []

    def send(r0, rows, c0, cols):
        win = (pl.ds(r0, rows), pl.ds(c0, cols))
        copies.append(pltpu.make_async_copy(x_s.at[win], o_hbm.at[win], sem_out.at[len(copies)]))
        copies[-1].start()

    def queue_halves(k):
        d0, t0 = ga_at(*turn[k])

        def emit(marks):
            def block(i, j):
                w = [ga_s.get(d0 + HB * i, d0 + HB * (i + 1), t0 + 3 * j + t) for t in range(3)]
                w = [pacer.tie(w[t], marks[t::3]) if i == j else w[t] for t in range(3)]
                return _halves(_cat(w, 1)).astype(F32)
            for r, v in enumerate(_lhs7([[block(i, j) for j in range(2)] for i in range(2)])):
                if r not in (2, 3):
                    gc_s.put(HB * (7 * (k % 2) + r), 0, v)
        pacer.collect("a", GAP["halves"], ("a", k), 3 * HB // 16, emit)

    def seventh(p, q):
        d0, t0 = ga_at(p, q)
        lhs = ga_s.get(d0, d0 + S // 4, t0 + NP - 1)
        rhs = [_halves(we_s.get(128 * (7 * p + q), 128 * (7 * p + q + 1), n)) for n in range(2)]

        def product(r0, rows, n):
            pacer.now += rows // 4
            return _dot(_rows(lhs, r0 // 2, (r0 + rows) // 2), rhs[n])
        return product

    def two_levels(p, q):
        d0, t0 = ga_at(p, q)
        w0 = 4 * 384 * q
        out = {}
        for i in range(2):
            rows = (d0 + HB * i, d0 + HB * (i + 1))
            c = pacer.dot(ga_s.get(*rows, t0 + 4, t0 + 6), wd_s.get(w0 + 512, w0 + 768, 0, 2), HB)
            for n in range(2):
                out[i, n] = _tile(c, n) + pacer.dot(ga_s.get(*rows, t0, t0 + 4), wd_s.get(w0, w0 + 512, n), HB)
        return out

    def three_levels(p, q, extra):
        k = turn.index((p, q))
        pacer.flush(("a", k))
        if k + 1 < len(turn):
            queue_halves(k + 1)
        d0, t0 = ga_at(p, q)
        w0 = 4 * 384 * (7 * (k // 7 % 3) + q)
        lhs = [ga_s.get(d0 + HB * (r - 2), d0 + HB * (r - 1), t0 + 3 * (r - 2), t0 + 3 * (r - 1)) if r in (2, 3)
               else gc_s.get(HB * (7 * (k % 2) + r), HB * (7 * (k % 2) + r + 1), 0, 3) for r in range(7)]
        rhs = [_halves(wd_s.get(w0 + 384 * (r // 2), w0 + 384 * (r // 2 + 1), r % 2)) for r in range(7)]
        last = seventh(p, q)
        out = {}
        for c in range(0, HB, ROWS):
            m = {}
            for r in ORDER1:
                m[r] = pacer.dot(_rows(lhs[r], c // 2, (c + ROWS) // 2), rhs[r], 3 * ROWS // 4)
                for i, n in _TERMS:
                    if r == _last(i, n):
                        v = _out4(m.get, i, n, ORDER1[::-1]) + last(HB * i + c, ROWS, n)
                        out.setdefault((i, n), []).append(v)
                for _ in range(0 if c else {1: 1, 2: 1, 5: 2}.get(r, 0)):
                    next(extra, None)
        return {c: _cat(v, 0) for c, v in out.items()}

    def inner(p, m):
        low[p] = {c: [[_out4(lambda q: m[q][c], i, j, ORDER1) for j in range(2)] for i in range(2)] for c in m[0]}

    def sevenths(p, m):
        for q in ORDER1:
            last = seventh(p, q)
            for i, n in m[q]:
                m[q][i, n] += last(HB * i, HB, n)
                yield
        inner(p, m)

    def queue_finish(hi, hj):
        have = [p for p in ORDER1 if p in low and p in _TERMS[hi, hj]]
        for i3, n in low[have[0]]:
            def emit(marks, i3=i3, n=n):
                def term(p):
                    v = _cat([_cat([_rows(w, QB * b, QB * (b + 1)) for w in low[p][i3, n][i]], 1)
                              for b in range(2) for i in range(2)], 0)
                    return pacer.tie(v, marks) if p == have[-1] else v
                o = _out4(term, hi, hj, have) * scale + _tile(b2, 4 * n + 2 * hj, 2)
                for b in range(2):
                    r0, c0 = (2 * i3 + b) * TB + HB * hi, 512 * n + 256 * hj
                    v = _rows(o, HB * b, HB * (b + 1)) + x_s[r0:r0 + HB, c0:c0 + 256].astype(F32)
                    if len(have) == len(_TERMS[hi, hj]):
                        x_s[r0:r0 + HB, c0:c0 + 256] = v.astype(BF)
                    else:
                        partial[i3, n, b] = v
            pacer.collect("f", GAP["finish_last" if len(low) == 6 else "finish"], ("f", hi, hj), 2 * HB // 16, emit)

    def send_block(hi, hj):
        for blk in range(NB):
            for n in range(2):
                send(blk * TB + HB * hi, HB, 512 * n + 256 * hj, 256)

    def send_last(m, blocks):
        wins = []
        for i, j in blocks:
            for i3, n in m[ORDER1[0]]:
                v = _out4(lambda q: m[q][i3, n], i, j, ORDER1[::-1])
                for b in range(2):
                    r0, c0 = (2 * i3 + b) * TB + QB * i, 512 * n + 128 * j
                    rest = lax.slice(partial[i3, n, b], (QB * i, 128 * j), (QB * (i + 1), 128 * (j + 1)))
                    x_s[r0:r0 + QB, c0:c0 + 128] = (_rows(v, QB * b, QB * (b + 1)) * scale + rest).astype(BF)
                    wins.append((r0, QB, c0, 128))
        for win in wins:
            send(*win)

    pacer.flush(("w2", 0))
    first = {}
    for q in ORDER1:
        if q == ORDER1[-1]:
            queue_halves(7)
        first[q] = two_levels(ORDER1[0], q)
    pacer.flush(("g", NP - 1))
    for k in range(1, 7):
        p = ORDER1[k]
        pacer.flush(("w2", k))
        if k == 2:
            split()
        if k == 6:
            pacer.flush(("f", 1, 0))
            pacer.flush(("f", 0, 1))
            send_block(1, 0)
            send_block(0, 1)
            split()
        else:
            queue_w2(k + 1)
        for c in {2: [(1, 0)], 4: [(0, 1)], 6: [(1, 1), (0, 0)]}.get(k, ()):
            queue_finish(*c)
        late = sevenths(ORDER1[0], first) if k == 1 else iter(())
        m = {}
        for q in ORDER1:
            if k == 6 and q == ORDER1[4]:
                pacer.flush(("f", 1, 1))
                pacer.flush(("f", 0, 0))
                send_last(m, [(1, 0), (0, 1)])
                send_block(1, 1)
            if k == 6 and q == ORDER1[6]:
                send_last(m, [(1, 1)])
            m[q] = three_levels(p, q, late)
        next(late, None)
        if k < 6:
            inner(p, m)
    send_last(m, [(0, 0)])
    for c in copies:
        c.wait()


@jax.jit
def pallas_sequential_preLN__sliding_block__mixer_channel_mlp__prompt_kernel(
        A_x, A_wqkv, A_wo, B_x, B_w1, B_b1, B_w2, B_b2):
    del B_x
    any_spec = pl.BlockSpec(memory_space=pl.ANY)
    out = pl.pallas_call(
        _kernel,
        out_shape=jax.ShapeDtypeStruct((S, D), BF),
        in_specs=[any_spec] * 7,
        out_specs=any_spec,
        scratch_shapes=[
            pltpu.VMEM((S, D), BF), pltpu.VMEM((D, D), BF), pltpu.VMEM((D, F), BF), pltpu.VMEM((F, D), BF),
            pltpu.VMEM((F,), BF), pltpu.VMEM((D,), BF),
            pltpu.VMEM((2 * TB, D), F32), pltpu.VMEM((512, 512), F32),
            pltpu.VMEM((3 * W, 256), I32), pltpu.VMEM((49 * S // 8, 256), I32),
            pltpu.VMEM((49 * 128 * 4, 256), I32), pltpu.VMEM((48384, 256), I32),
            pltpu.SemaphoreType.DMA((19,)), pltpu.SemaphoreType.DMA((14 * NB,)),
        ],
        compiler_params=pltpu.CompilerParams(vmem_limit_bytes=127 << 20),
        name="fused_block",
    )(A_x.reshape(S, D), A_wqkv, A_wo, B_w1, B_b1, B_w2, B_b2)
    return out.reshape(1, S, D)
```

```python
import math

import jax
import jax.numpy as jnp
from jax import lax
import jax.experimental.pallas as pl
import jax.experimental.pallas.tpu as pltpu

S, D, F = 2048, 1024, 3584
DH, W = 32, 256
EPS = 1e-5
TB = 512
NB = S // TB
HB, QB = TB // 2, TB // 4
NP = F // 512
BF, F32, I32 = jnp.bfloat16, jnp.float32, jnp.int32

GS = (math.sqrt(2.0 / math.pi) * 0.044715) ** (1.0 / 3.0)
GK = math.sqrt(2.0 / math.pi) / GS

GAP = {
    "exp": 25, "o": 150, "x": (None, 116, 410, 410), "h": (130, 113, 113, 113),
    "wa": {(0, 0): 27, (0, 1): 31, (0, 2): 31, (1, 0): 50, (1, 1): 83, (1, 2): 135},
    "wo": 150, "w1": (100, 45, 45, 19, 19, 108, 108), "w2": (66, 66, 69.5) + (60.5,) * 4,
    "gelu": (48,) * (NP - 1) + (41.5,), "halves": 32, "finish": 150, "finish_last": 24,
}
COST = {"exp": 9, "o": 9, "xc": 9, "hc": 1, "w": 9, "g": 14, "a": 7, "f": 9}
COST_FIRST = {"xc": 24, "hc": 1, "w": 24}
W1_WHEN = {"qkv": (0,), "wo": (1, 2), 0: (3, 4), 1: (5,), 2: (6,)}
ROWS = 64
TRANSPOSE_TIME = 900
REDUCE_TIME = 180
NORM_TIME = 200
SCORE_PACE = 0.8
EARLY = ((2, 4), (3, 6))


def _cat(xs, axis):
    return xs[0] if len(xs) == 1 else lax.concatenate(xs, axis)


def _rows(x, r0, r1):
    return lax.slice_in_dim(x, r0, r1, axis=0)


def _tile(x, t, n=1):
    return lax.slice_in_dim(x, 128 * t, 128 * (t + n), axis=1)


def _words(x):
    return pltpu.bitcast(x.astype(BF), I32)


def _halves(w):
    return pltpu.bitcast(w, BF) if w.dtype == I32 else w


def _dot(a, b):
    return lax.dot_general(_halves(a), _halves(b), (((1,), (0,)), ((), ())), preferred_element_type=F32)


def _dot_nt(a, b):
    return lax.dot_general(_halves(a), _halves(b), (((1,), (1,)), ((), ())), preferred_element_type=F32)


def _layernorm(x, scales=None):
    m = jnp.mean(x, axis=-1, keepdims=True)
    yield
    xc = x - m
    v = jnp.mean(xc * xc, axis=-1, keepdims=True)
    yield
    r = lax.rsqrt(v + EPS)
    if scales is None:
        return xc * r
    n = x.shape[1] // 128 // len(scales)
    rs = {c: r * c for c in scales}
    return _cat([_tile(xc, n * i, n) * rs[c] for i, c in enumerate(scales)], 1)


def _lhs7(a):
    (a11, a12), (a21, a22) = a
    return [a11 + a22, a21 + a22, a11, a22, a11 + a12, a21 - a11, a12 - a22]


def _rhs7(b):
    (b11, b12), (b21, b22) = b
    return [b11 + b22, b11, b12 - b22, b21 - b11, b22, b11 + b12, b21 + b22]


_TERMS = {(0, 0): {0: 1, 3: 1, 4: -1, 6: 1}, (0, 1): {2: 1, 4: 1},
          (1, 0): {1: 1, 3: 1}, (1, 1): {0: 1, 1: -1, 2: 1, 5: 1}}
ORDER1 = (1, 3, 2, 4, 5, 0, 6)
ORDER2 = (ORDER1, (6, 1, 3, 2, 4, 5, 0))


def _out4(m, i, j, order):
    acc = None
    for p in reversed(order):
        sign = _TERMS[i, j].get(p)
        if sign and acc is None:
            acc = m(p) if sign > 0 else -m(p)
        elif sign:
            acc = acc + m(p) if sign > 0 else acc - m(p)
    return acc


def _last(i, j):
    return [p for p in ORDER1 if p in _TERMS[i, j]][-1]


_ROW = (1.0, math.sqrt(3.0), math.sqrt(3.0), 3.0)
_COL = _ROW[::-1]
BAL1 = (0, 1, 2, 4, 6, 3, 5)
BAL2 = ((1, 2, 4, 6, 3, 5, 0), BAL1)


def _bal_lhs7(a):
    (a11, a12), (a21, a22) = a
    s, t = a11 + a22, a12 + a21
    return [s, a11 - a12, a11 + a12, s - t, a12 - a22, s + t, a12 + a22]


def _bal_rhs7(b):
    (b11, b12), (b21, b22) = b
    s, t = b11 + b22, b12 + b21
    return [s + s, b12 - b22, b12 + b22, b11 + b12, s + t, b11 - b12, s - t]


def _bal_out(m, order):
    c12, e = m[1] + m[2], m[1] - m[2]
    c21 = (c12 - (m[4] + m[6])) + (m[5] - m[3])
    if order[0] == 0:
        d = e + m[0]
        return [[d + (m[4] - m[6]), c12], [c21, d - (m[3] + m[5])]]
    return [[(e + (m[4] - m[6])) + m[0], c12], [c21, (e - (m[3] + m[5])) + m[0]]]


STD_TURN = (ORDER1, ((0, 0), (1, 1)))
BAL_TURN = ((1, 2, 3, 5, 0, 4, 6), ((0, 0), (0, 1)))


def _nested(f, a, hold=lambda q, k, v: v):
    low = {(hi, hj): f([[a[2 * hi + i][2 * hj + j] for j in range(2)] for i in range(2)])
           for hi in range(2) for hj in range(2)}
    return {(p, q): v for q in range(7)
            for p, v in enumerate(f([[hold(q, (hi, hj), low[hi, hj][q]) for hj in range(2)] for hi in range(2)]))}


def _lane_bits(shape):
    lane = lax.broadcasted_iota(I32, shape, 1)
    return (lane & 32) == 0, (lane & 64) == 0


def _butterfly(v, b0, b1):
    u = [lax.select(b0, v[i], v[i ^ 1]) for i in range(4)]
    return [lax.select(b1, u[i], u[i ^ 2]) for i in range(4)]


class _Pacer:
    def __init__(self):
        self.masks = {}
        self.now = 0.0
        self.mark = None
        self.busy = 0.0
        self.free = {}
        self.events = []
        self.dues = []

    def tie(self, value, marks):
        known = [m for m in marks if m is not None]
        if not known:
            return value
        if value.shape not in self.masks:
            lane = lax.broadcasted_iota(I32, value.shape, 1) & 127
            self.masks[value.shape] = lane * lane == 2
        n = value.shape[0] // 8 // len(marks)
        wait = _cat([known[-1] if m is None else m for m in marks for _ in range(n)], 0)
        if wait.dtype != value.dtype:
            wait = pltpu.bitcast(wait, value.dtype)
        return lax.select(self.masks[value.shape], _cat([wait] * (value.shape[1] // 128), 1), value)

    def due(self, value, delay):
        self.dues.append((self.now + delay, pltpu.bitcast(value, I32)))

    def at(self, t, tag, job):
        self.events.append((t, tag, job))
        self.events.sort(key=lambda e: e[0])

    def add(self, lane, gap, tag, job, delay=0):
        t = max(self.now + delay, self.free.get(lane, 0.0))
        self.free[lane] = t + gap
        self.at(t, tag, job)

    def collect(self, lane, gap, tag, n, then, delay=0, group=0):
        marks = []

        def job():
            marks.append(self.mark)
            if len(marks) == n:
                then(marks)
            return COST_FIRST[lane] if group and len(marks) % group == 1 else COST[lane]
        for _ in range(n):
            self.add(lane, gap, tag, job, delay)

    def stepwise(self, tag, steps):
        def job():
            if next(steps, self) is not self:
                self.at(self.now + REDUCE_TIME, tag, job)
            return 1
        return job

    def tick(self, r, cycles):
        n = r.shape[0] // 8
        for i in range(n):
            self.now += cycles / n
            if self.events and max(self.busy, self.events[0][0]) <= self.now:
                self.mark = lax.slice(r, (8 * i, 0), (8 * i + 8, 128))
                self.busy = self.now + self.events.pop(0)[2]()
        self.mark = None

    def flush(self, tag):
        while tag in [e[1] for e in self.events]:
            t, _, job = self.events.pop([e[1] for e in self.events].index(tag))
            self.now, now = t, self.now
            job()
            self.now = now

    def dot(self, lhs, rhs, cycles, last=True):
        n = lhs.shape[0]
        for t, v in self.dues:
            if t < self.now + cycles:
                i = 8 * max(0, int((t - self.now) * (n // 8) / cycles))
                parts = [_rows(lhs, 0, i)] if i else []
                parts.append(self.tie(_rows(lhs, i, i + 8), [v]))
                lhs = _cat(parts + ([_rows(lhs, i + 8, n)] if i + 8 < n else []), 0)
        r = _dot(lhs, rhs)
        if last:
            self.dues = [d for d in self.dues if d[0] >= self.now + cycles]
            self.tick(r, cycles)
        return r


class _Words:
    def __init__(self, pool, start, rows, tiles):
        self.pool, self.start, self.rows = pool, start, rows // 2
        self.end = start + self.rows * ((tiles + 1) // 2)
        assert self.end <= pool.shape[0]

    def _window(self, r0, n, t, k):
        r = self.start + (t // 2) * self.rows + r0 // 2
        return slice(r, r + n), slice(128 * (t % 2), 128 * (t % 2 + k))

    def _runs(self, t0, t1):
        while t0 < t1:
            k = 2 if t0 % 2 == 0 and t0 + 1 < t1 else 1
            yield t0, k
            t0 += k

    def get(self, r0, r1, t0, t1=None):
        return _cat([self.pool[self._window(r0, (r1 - r0) // 2, t, k)] for t, k in self._runs(t0, t1 or t0 + 1)], 1)

    def put(self, r0, t0, x):
        runs = list(self._runs(t0, t0 + x.shape[1] // 128))
        for t, k in runs:
            part = x if len(runs) == 1 else _tile(x, t - t0, k)
            self.pool[self._window(r0, x.shape[0] // 2, t, k)] = _words(part)


def _interleave(a, na, b, nb):
    ia = ib = 0
    while ia < na or ib < nb:
        if ib >= nb or (ia < na and ia * nb <= ib * na):
            next(a)
            ia += 1
        else:
            next(b)
            ib += 1


def _kernel(x_hbm, wqkv_hbm, wo_hbm, w1_hbm, b1_hbm, w2_hbm, b2_hbm, o_hbm,
            x_s, wo_s, w1_s, w2_s, b1_s, b2_s, y_s, o_s, p_pool, ya_pool, wb_pool, pool, sem_in, sem_out):
    pacer = _Pacer()
    sems = iter(range(sem_in.shape[0]))

    def copy(src, dst):
        return pltpu.make_async_copy(src, dst, sem_in.at[next(sems)])

    def wqkv_copy(m, c0, n):
        return copy(wqkv_hbm.at[:, pl.ds(m * D + c0, n)], w2_s.at[pl.ds(m * D, D), pl.ds(c0, n)])

    def row_copy(src, dst, r0, r1):
        return copy(src.at[pl.ds(r0, r1 - r0)], dst.at[pl.ds(r0, r1 - r0)])

    first_rows = (0, HB, QB, HB + QB)
    stages = [[row_copy(x_hbm, x_s, r, r + QB)] for r in first_rows] + [
        [wqkv_copy(0, 0, 128)],
        [wqkv_copy(0, 128, 384)],
        [wqkv_copy(1, 0, 512)],
        [wqkv_copy(2, 0, 512)],
        [wqkv_copy(0, 512, 512)],
        [wqkv_copy(1, 512, 512), wqkv_copy(2, 512, 512), row_copy(x_hbm, x_s, TB, 2 * TB)],
    ]
    rest = [row_copy(x_hbm, x_s, 2 * TB, S), copy(b1_hbm, b1_s), copy(b2_hbm, b2_s), copy(wo_hbm, wo_s)]
    w1_copy = copy(w1_hbm, w1_s)
    w2_copies = [row_copy(w2_hbm, w2_s, r, r + F // 2) for r in (0, F // 2)]
    for stage in stages + [rest]:
        for c in stage:
            c.start()

    def landed():
        for c in stages.pop(0):
            c.wait()

    lane = lax.broadcasted_iota(I32, (32, 128), 1)
    row = lax.broadcasted_iota(I32, (32, 128), 0)
    top_valid = row > (lane & 31)
    lane16 = lax.broadcasted_iota(I32, (16, 128), 1)
    row16 = lax.broadcasted_iota(I32, (16, 128), 0)
    top_words = (jnp.where(2 * row16 > (lane16 & 31), 0xFFFF, 0)
                 | jnp.where(2 * row16 + 1 > (lane16 & 31), -0x10000, 0))
    low_words = ~top_words

    zero = jnp.clip((lane16 * lane16)[0, 0], 0, 1) * 8
    for buf in (y_s, o_s, p_pool, ya_pool, wb_pool, pool):
        buf[pl.ds(zero, 8), 0:128] = jnp.zeros((8, 128), buf.dtype)
    p_s = _Words(p_pool, 0, 3 * W, 4)
    xa_s = _Words(pool, 0, 2 * 49 * QB, 2)
    oa_s = _Words(pool, xa_s.end, 7 * S // 2, 4)
    q_s = _Words(pool, oa_s.end, 2 * TB, 8)
    k_s = _Words(pool, q_s.end, S, 8)
    vt_s = _Words(pool, k_s.end, D, S // 128)
    wa_s = _Words(pool, vt_s.end, 49 * 256, 6)
    xn_s = _Words(pool, wa_s.end, TB, 8)
    xb_s = _Words(pool, xn_s.end, 7 * HB, 4)
    wc_s = _Words(pool, wa_s.end, 7 * 512, 4)
    ya_s = _Words(ya_pool, 0, 49 * S // 4, 2)
    wb_s = _Words(wb_pool, 0, 49 * 256, NP)
    ga_s = _Words(pool, 0, 25 * S // 4, 2 * NP)
    gc_s = _Words(pool, ga_s.end, 14 * HB, 3)
    we_s = _Words(wb_pool, 0, 49 * 128, 2)
    wd_s = _Words(wb_pool, we_s.end, 21 * 4 * 384, 2)

    def split(wait=(), start=()):
        for c in wait:
            c.wait()
        for c in start:
            c.start()

        @pl.when(zero != 0)
        def _():
            pool[0:8, 0:128] = jnp.zeros((8, 128), I32)

    def x_rows(r0):
        x = x_s[r0:r0 + 8, :].astype(F32)
        return _cat([pacer.tie(_tile(x, 0), [pacer.mark]), _tile(x, 1, 7)], 1)

    def queue_operands(lane, gap, tag, steps, combine, turn, block, put, delay=0):
        order, held = turn

        def emit(marks):
            def hold(q, k, v):
                return pacer.tie(v, marks[order.index(q)::7]) if k in held else v
            for (p, q), v in _nested(combine, [[block(a, b) for b in range(4)] for a in range(4)], hold).items():
                put(7 * p + q, v)
        pacer.collect(lane, gap, tag, 7 * steps, emit, delay, 7)

    def queue_rows(lane, blk, group, normed, combine, turn, dest, row0):
        gap = GAP[lane][blk]
        done = []

        def steps(i, r):
            y = yield from normed(i, r)
            r0 = r // 16 * 16
            y0 = TB * (blk % 2) + r0
            y_s[y0 + QB * i + r - r0:y0 + QB * i + r - r0 + 8, :] = y
            done.append(_tile(y, 0))
            if len(done) % group == 0:
                pacer.due(sum(done[1 - group:], done[-group]), NORM_TIME)
            if len(done) % 8 == 0:
                for c in range(2):
                    queue_operands(
                        lane + "c", gap * 8 / 15, (lane, blk), 1, combine, turn,
                        lambda a, b, c=c: y_s[y0 + QB * a:y0 + QB * a + 16, 256 * b + 128 * c:256 * b + 128 * (c + 1)],
                        lambda k, v, c=c: dest.put(row0(k) + r0, c, v), NORM_TIME + 50)
        pacer.flush((lane, blk - 2))
        for r in range(0, QB, 16):
            for i in range(4):
                for rr in (r, r + 8):
                    pacer.add(lane, gap, (lane, blk), pacer.stepwise((lane, blk), steps(i, rr)))

    qscale = (DH ** -0.5) * math.log2(math.e)
    count = [0, 0]
    bits = {n: _lane_bits((n, 128)) for n in (1, 16, 32, 64, 128, 192)}
    nought = jnp.zeros((16, 128), I32)

    def queue_x(blk):
        queue_rows("x", blk, 2 if blk > 1 else 4,
                   lambda i, r: _layernorm(x_rows(blk * TB + i * QB + r), [_ROW[i] * c for c in _COL]),
                   _bal_lhs7, BAL_TURN, xa_s, lambda k: (blk % 2 * 49 + k) * QB)

    def queue_wa(j, m):
        def block(a, b):
            r0, c0 = m * D + 256 * a, 512 * j + 256 * (b // 2)
            return _tile(w2_s[r0:r0 + 256, c0:c0 + 256].astype(F32), b % 2) * (_ROW[a] * _COL[b])
        queue_operands("w", GAP["wa"][j, m], ("wa", j, m), 16, _bal_rhs7, BAL_TURN, block,
                       lambda k, v: wa_s.put(256 * k, 3 * j + m, v))

    def put_qkv(m, r0, g, c):
        if m == 0:
            q_s.put(r0 % (2 * TB), g, c)
        elif m == 1:
            k_s.put(r0, g, c)
        else:
            c = c.T
            vt_s.put(128 * g, r0 // 128, c)
        return lax.slice(c, (c.shape[0] - 8, c.shape[1] - 128), c.shape)

    def first_products(j, m):
        for g in range(4 * j, 4 * j + 4):
            if (m, g) == (0, 1):
                landed()
                queue_wa(0, 0)
            c = pacer.dot(xn_s.get(0, TB, 0, 4), w2_s[m * D:m * D + 512, 128 * g:128 * (g + 1)], TB)
            yield
            c += pacer.dot(xn_s.get(0, TB, 4, 8), w2_s[m * D + 512:(m + 1) * D, 128 * g:128 * (g + 1)], TB)
            last = put_qkv(m, 0, g, c * qscale if m == 0 else c)
            if m == 2:
                pacer.due(last, TRANSPOSE_TIME)
            yield

    def first_one_level(m):
        for g in (0, 2):
            w = w2_s[m * D:(m + 1) * D, 128 * g:128 * (g + 2)].astype(F32)
            rhs = _rhs7([[_tile(_rows(w, 512 * a, 512 * (a + 1)), b) for b in range(2)] for a in range(2)])
            prod = {}
            for p in ORDER1:
                prod[p] = pacer.dot(xb_s.get(HB * p, HB * (p + 1), 0, 4), rhs[p].astype(BF), HB)
                for i, b in _TERMS:
                    if p == _last(i, b):
                        last = put_qkv(m, HB * i, g + b, _out4(prod.get, i, b, ORDER1))
                        if m == 2:
                            pacer.due(last, TRANSPOSE_TIME)

    def qkv_products(blk, j):
        for m in range(3):
            pacer.flush(("wa", j, m))
            low = {}
            for p in BAL1:
                order = BAL2[count[0] % 2]
                count[0] += 1
                prod = {}
                for q in order:
                    k = 7 * p + q
                    o = (blk % 2 * 49 + k) * QB
                    prod[q] = pacer.dot(xa_s.get(o, o + QB, 0, 2), wa_s.get(256 * k, 256 * (k + 1), 3 * j + m),
                                        QB * (876 - 288 * SCORE_PACE) / 588, count[1] % 2)
                    count[1] += 1
                    if q == order[-1]:
                        low[p] = _bal_out(prod, order)
                        if p == BAL1[-1]:
                            finish_qkv(blk, j, m, low)
                    if count[1] % 2 == 0:
                        yield

    def finish_qkv(blk, j, m, low):
        c = {}
        for i in range(2):
            for k in range(2):
                t = _bal_out({p: low[p][i][k] for p in BAL1}, BAL1)
                c.update({(2 * hi + i, 2 * hj + k): t[hi][hj] for hi in range(2) for hj in range(2)})
        turn = ((0, 1), (0, 0), (1, 0), (1, 1))
        for hi, hj in turn:
            for i, k in turn:
                a, b = 2 * hi + i, 2 * hj + k
                scale = (qscale if m == 0 else 1.0) / (12 * _ROW[a] * _COL[b])
                last = put_qkv(m, blk * TB + a * QB, 4 * j + b, c[a, b] * scale)
        if m == 2:
            pacer.due(last, TRANSPOSE_TIME)

    def scores(sb, g, slot, turn=(0, 1, 2, 3)):
        j0 = max(0, 8 - 4 * sb)
        ss, ms = {}, {}
        b0, b1 = bits[16]
        for t in turn:
            qt = q_s.get(128 * (sb % 8) + 32 * t, 128 * (sb % 8) + 32 * (t + 1), g)
            q2 = [lax.select(b0, qt, nought), lax.select(b0, nought, qt)]
            q4 = [lax.select(b1, v, nought) for v in q2] + [lax.select(b1, nought, v) for v in q2]
            lo = max(j0, t)
            keys = k_s.get(128 * sb - W + 32 * lo, 128 * sb - W + 32 * (t + 9), g)
            s = _dot_nt(keys, _cat([q4[c ^ t] for c in range(4)], 0))
            n = s.shape[0]
            if t == 3:
                pacer.tick(s, n * SCORE_PACE)
            first = _rows(s, 0, 32) if lo == t else jnp.full((32, 128), -jnp.inf, F32)
            body = [_rows(s, 32 if lo == t else 0, n - 32)] if n > 32 else []
            ss[t] = _cat(body + [lax.select(top_valid, first, _rows(s, n - 32, n))], 0)
            ms[t] = jnp.broadcast_to(jnp.max(ss[t], axis=0, keepdims=True), (8, 128))
        todo = [(j, t) for j in range(j0, 12) for t in range(4) if 0 <= j - t < 8 or (j - t == 8 and t < j0)]
        sums = []

        def emit(marks):
            ends = [ss[t].shape[0] - (0 if j == t else 32 * (8 + t - j)) for j, t in todo]
            s = _cat([_rows(ss[t], e - 32, e) for (_, t), e in zip(todo, ends)], 0)
            p = jnp.exp2(s - pacer.tie(_cat([ms[t] for _, t in todo for _ in range(4)], 0), marks))
            for t in range(4):
                pt = _cat([_rows(p, 32 * k, 32 * (k + 1)) for k, (_, u) in enumerate(todo) if u == t], 0)
                sums.append(jnp.sum(pt, axis=0, keepdims=True))
                p_s.put(W * slot, t, pt)
        pacer.collect("exp", GAP["exp"], (sb, g), len(todo), emit)
        return sums

    def values(sb, g, slot, sums):
        j0 = max(0, 8 - 4 * sb)
        pacer.flush((sb, g))
        inv = _butterfly([pltpu.reciprocal(l, full_range=False) for l in sums], *bits[1])
        v = []
        for t in range(4):
            n = min(8, 9 + t - j0)
            w = p_s.get(W * slot, W * slot + 32 * n, t)
            parts = [w]
            if t >= j0:
                edge = _rows(w, 0, 16)
                parts = [nought] * (t - j0) + [edge & top_words, _rows(w, 16, 16 * n), edge & low_words]
            v.append(_cat(parts + [nought] * (3 - t), 0))
        heads = _butterfly(v, *bits[v[0].shape[0]])
        outs = [None] * 4
        for k in range(3 - j0 // 4):
            for h in range(4):
                vt = vt_s.get(128 * g + DH * h, 128 * g + DH * (h + 1), sb - 2 + j0 // 4 + k)
                o = _dot(vt, _rows(heads[h], 64 * k, 64 * (k + 1)))
                outs[h] = o if k == 0 else outs[h] + o
        ot = _cat([o * i for o, i in zip(outs, inv)], 0).T
        pacer.due(_rows(ot, 120, 128), TRANSPOSE_TIME)
        r0, c0 = 256 * (sb % 2), 256 * (g // 2 % 2)
        pacer.flush(("o", r0, c0))
        a0, b0 = r0 + 128 * (sb % 4 // 2), c0 + 128 * (g % 2)
        o_s[a0:a0 + 128, b0:b0 + 128] = _cat(_butterfly([_rows(ot, r, r + 32) for r in range(0, 128, 32)], *bits[32]), 0)
        if sb % 4 >= 2 and g % 2:
            def emit(marks):
                a = [[o_s[r0 + 128 * i:r0 + 128 * (i + 1), c0 + 128 * b:c0 + 128 * (b + 1)] for b in range(2)]
                     for i in range(2)]
                for i in range(2):
                    a[i][i] = pacer.tie(a[i][i], marks)
                for p, v in enumerate(_lhs7(a)):
                    oa_s.put(((sb // 4) * 7 + p) * HB + 128 * (sb % 2), g // 2, v)
            pacer.collect("o", GAP["o"], ("o", r0, c0), 8, emit, TRANSPOSE_TIME + 50)

    def attention():
        units = [(4 * blk + s, 4 * j + g + b) for blk in range(NB) for j in range(2) for g in (2, 0)
                 for s in (0, 2, 1, 3) for b in range(2)]
        prev = None
        for n, u in enumerate(units):
            if u[0] >= 2:
                sums = scores(*u, n % 3)
            elif n % 2 == 0:
                sums = scores(*u, n % 3)
                ahead = scores(*units[n + 1], (n + 1) % 3, (3, 2, 1, 0))
            else:
                sums = ahead
            yield
            if prev:
                values(*prev)
            prev = (*u, n % 3, sums)
            yield
        yield
        values(*prev)
        yield

    def queue_wo(n):
        def emit(marks):
            def block(a, b):
                w = _cat([wo_s[128 * k:128 * (k + 1), 256 * n:256 * (n + 1)] for k in range(a, 8, 2)], 0)
                w = _tile(w.astype(F32), b)
                return pacer.tie(w, marks) if a == b else w
            for p, v in enumerate(_rhs7([[block(a, b) for b in range(2)] for a in range(2)])):
                wc_s.put(512 * p, n, v)
        pacer.collect("w", GAP["wo"], "wo", 32, emit)

    def wo_products(blk):
        c = {}
        for n in range(4):
            prod = {}
            for p in ORDER1:
                o = (blk * 7 + p) * HB
                prod[p] = pacer.dot(oa_s.get(o, o + HB, 0, 4), wc_s.get(512 * p, 512 * (p + 1), n), HB)
                if p == ORDER1[-1]:
                    for i in range(2):
                        for b in range(2):
                            c[i, 2 * n + b] = _out4(prod.get, i, b, ORDER1)
                    if n == 3:
                        queue_h(blk, _cat([_cat([c[i, t] for t in range(8)], 1) for i in range(2)], 0))
                yield

    def queue_h(blk, o):
        hs = {}

        def normed(i, r):
            r0 = blk * TB + i * QB + r
            h = hs[i, r] = x_rows(r0) + _rows(o, i * QB + r, i * QB + r + 8)
            if r % 16:
                x_s[r0 - 8:r0 + 8, :] = _cat([hs[i, r - 8], h], 0).astype(BF)
            return (yield from _layernorm((yield from _layernorm(h)), (GS,)))
        queue_rows("h", blk, 4, normed, _lhs7, STD_TURN, ya_s, lambda k: k * (S // 4) + blk * QB)

    def queue_w1(n):
        def block(a, b):
            c0 = 512 * n + 256 * (b // 2)
            return _tile(w1_s[256 * a:256 * (a + 1), c0:c0 + 256].astype(F32), b % 2)
        queue_operands("w", GAP["w1"][n], ("w1", n), 16, _rhs7, STD_TURN, block,
                       lambda k, v: wb_s.put(256 * k, n, v))

    ga = attention()
    xn = {}
    for r in first_rows:
        landed()

        def steps(r=r):
            xn[r] = yield from _layernorm(x_s[r:r + QB, :].astype(F32))
        list(steps())
        xn_s.put(r, 0, xn[r])
        if r >= HB:
            for p, v in enumerate(_lhs7([[_tile(xn[i], 4 * k, 4) for k in range(2)] for i in (r - HB, r)])):
                xb_s.put(HB * p + r - HB, 0, v)
    landed()
    list(first_products(0, 0))
    landed()
    queue_wa(0, 1)
    first_one_level(1)
    landed()
    queue_wa(0, 2)
    first_one_level(2)
    landed()
    queue_wa(1, 0)
    _interleave(first_products(1, 0), 8, ga, 17)
    landed()
    queue_x(1)
    queue_wa(1, 1)
    _interleave((None for m in (1, 2) for _ in first_products(1, m)), 16, ga, 14)
    for blk in range(1, NB):
        pacer.flush(("x", blk))
        if blk == 1:
            queue_wa(1, 2)
            split(wait=rest, start=[w1_copy])
        if blk < NB - 1:
            queue_x(blk + 1)
        else:
            split(wait=[w1_copy])
            for n in range(4):
                queue_wo(n)
            for n in W1_WHEN["qkv"]:
                queue_w1(n)
        for j in range(2):
            gp = qkv_products(blk, j)
            _interleave(gp, (147 + count[1] % 2) // 2, ga, 32)
            next(gp, None)
    pacer.flush("wo")
    for n in W1_WHEN["wo"]:
        queue_w1(n)
    _interleave(wo_products(0), 28, ga, 17)
    _interleave(wo_products(1), 28, ga, 18)
    split(start=w2_copies[:1])
    list(wo_products(2))
    for r0 in (0, 256):
        for c0 in (0, 256):
            pacer.flush(("o", r0, c0))
    list(wo_products(3))

    b1 = b1_s[...].astype(F32).reshape(1, F) * GS
    b2 = b2_s[...].astype(F32).reshape(1, D)

    def ga_at(p, q):
        k = 7 * p + q
        return k // 2 * (S // 4), k % 2 * NP

    def queue_gelu(n, low):
        keys = [(i, j, hj) for i, j in ((0, 1), (1, 0), (0, 0), (1, 1)) for hj in range(2)]

        def emit(marks):
            zs = []
            for k, (i, j, hj) in enumerate(keys):
                m = {p: low[p][i][j] for p in ORDER1}
                both = 3 - hj
                bias = jnp.broadcast_to(_tile(b1, 4 * n + 2 * hj + j), (S // 4, 128))
                m[both] = m[both] + pacer.tie(bias, marks[k::8])
                zs += [_out4(m.get, hi, hj, [p for p in ORDER1 if p != both] + [both]) for hi in range(2)]
            z = _cat([_rows(v, r, r + 16) for r in range(0, S // 4, 16) for v in zs], 0)
            g = z * jnp.tanh(z * (z * z + GK)) + z
            a = [[None] * 4 for _ in range(4)]
            for k, (i, j, hj) in enumerate(keys):
                for hi in range(2):
                    a[2 * hi + i][2 * hj + j] = _cat([_rows(g, 16 * (r + 2 * k + hi), 16 * (r + 2 * k + hi + 1))
                                                      for r in range(0, S // 4, 16)], 0)
            for (p, q), v in _nested(_lhs7, a).items():
                d0, t0 = ga_at(p, q)
                ga_s.put(d0, t0 + n, v)
        pacer.collect("g", GAP["gelu"][n], ("g", n), 8 * S // 64, emit)

    def queue_w2(k):
        p = ORDER1[k]

        def inner(positions, n):
            def block(a, b):
                c0 = 512 * n + 256 * (b // 2)
                w = [w2_s[512 * t + 128 * a:512 * t + 128 * (a + 1), c0:c0 + 256].astype(F32) for t in positions]
                return _tile(_cat(w, 0), b % 2)
            return _rhs7([[_rhs7([[block(2 * hi + i, 2 * hj + j) for hj in range(2)] for hi in range(2)])[p]
                           for j in range(2)] for i in range(2)])

        def emit(marks):
            low = [[inner(range(3 * i, 3 * i + 3), n) for n in range(2)] for i in range(2)]
            for q in range(7):
                v = [[low[i][n][q] for n in range(2)] for i in range(2)]
                for i in range(2):
                    for n in (i,) if k else range(2):
                        v[i][n] = pacer.tie(v[i][n], marks[ORDER1.index(q)::7])
                for r, w in enumerate(_rhs7(v) if k else v[0] + v[1]):
                    wd_s.put(384 * (4 * (7 * (k % 3) + q) + r // 2), r % 2, w)

        def emit_seventh(marks):
            for n in range(2):
                for q, w in enumerate(inner([NP - 1], n)):
                    we_s.put(128 * (7 * p + q), n, pacer.tie(w, marks[n::2]))
        pacer.collect("w", GAP["w2"][k], ("w2", k), 16, emit_seventh)
        pacer.collect("w", GAP["w2"][k], ("w2", k), 7 * 24, emit, 0, 7)

    def w1_products(n, p, b0, b1):
        order = ORDER2[count[0] % 2]
        count[0] += 1
        m = {}
        for q in order:
            k = 7 * p + q
            rhs = wb_s.get(256 * k, 256 * (k + 1), n)
            r0, r1 = k * (S // 4) + b0 * QB, k * (S // 4) + b1 * QB
            if (p, q, b1) == (ORDER1[-1], order[-1], NB):
                rm = (r0 + r1) // 2
                m[q] = _cat([pacer.dot(ya_s.get(r0, rm, 0, 2), rhs, rm - r0, False),
                             pacer.dot(ya_s.get(rm, r1, 0, 2), rhs, rm - r0)], 0)
            else:
                m[q] = pacer.dot(ya_s.get(r0, r1, 0, 2), rhs, r1 - r0, count[1] % 2)
            count[1] += 1
        return m, order

    low = None
    for n in range(NP):
        pacer.flush(("w1", n))
        if n in (1, 5):
            pacer.flush(("g", n - 2))
            split(wait=w2_copies if n == 5 else (), start=w2_copies[1:] if n == 1 else ())
        if n:
            queue_gelu(n - 1, low)
        if n >= NP - 2:
            queue_w2(n - NP + 2)
        count[:] = [0, 0]
        done = {p: (0, []) for p in ORDER1}
        if n == 0:
            for upto, some in EARLY:
                for b in range(upto):
                    pacer.flush(("h", b))
                for p in ORDER1[:some]:
                    done[p] = (upto, done[p][1] + [w1_products(n, p, done[p][0], upto)[0]])
            pacer.flush(("h", NB - 1))
            pacer.dues = []
        for k in W1_WHEN.get(n, ()):
            queue_w1(k)
        low = {}
        for p in ORDER1:
            tail, order = w1_products(n, p, done[p][0], NB)
            m = {q: _cat([v[q] for v in done[p][1] + [tail]], 0) for q in order}
            low[p] = [[_out4(m.get, i, j, order) for j in range(2)] for i in range(2)]
    for n in range(NP - 1):
        pacer.flush(("g", n))
    queue_gelu(NP - 1, low)

    turn = [(p, q) for p in ORDER1 for q in ORDER1]
    scale = 0.5 / GS
    low, partial, copies = {}, {}, []

    def send(r0, rows, c0, cols):
        win = (pl.ds(r0, rows), pl.ds(c0, cols))
        copies.append(pltpu.make_async_copy(x_s.at[win], o_hbm.at[win], sem_out.at[len(copies)]))
        copies[-1].start()

    def queue_halves(k):
        d0, t0 = ga_at(*turn[k])

        def emit(marks):
            def block(i, j):
                w = [ga_s.get(d0 + HB * i, d0 + HB * (i + 1), t0 + 3 * j + t) for t in range(3)]
                w = [pacer.tie(w[t], marks[t::3]) if i == j else w[t] for t in range(3)]
                return _halves(_cat(w, 1)).astype(F32)
            for r, v in enumerate(_lhs7([[block(i, j) for j in range(2)] for i in range(2)])):
                if r not in (2, 3):
                    gc_s.put(HB * (7 * (k % 2) + r), 0, v)
        pacer.collect("a", GAP["halves"], ("a", k), 3 * HB // 16, emit)

    def seventh(p, q):
        d0, t0 = ga_at(p, q)
        lhs = ga_s.get(d0, d0 + S // 4, t0 + NP - 1)
        rhs = [_halves(we_s.get(128 * (7 * p + q), 128 * (7 * p + q + 1), n)) for n in range(2)]

        def product(r0, rows, n):
            pacer.now += rows // 4
            return _dot(_rows(lhs, r0 // 2, (r0 + rows) // 2), rhs[n])
        return product

    def two_levels(p, q):
        d0, t0 = ga_at(p, q)
        w0 = 4 * 384 * q
        out = {}
        for i in range(2):
            rows = (d0 + HB * i, d0 + HB * (i + 1))
            c = pacer.dot(ga_s.get(*rows, t0 + 4, t0 + 6), wd_s.get(w0 + 512, w0 + 768, 0, 2), HB)
            for n in range(2):
                out[i, n] = _tile(c, n) + pacer.dot(ga_s.get(*rows, t0, t0 + 4), wd_s.get(w0, w0 + 512, n), HB)
        return out

    def three_levels(p, q, extra):
        k = turn.index((p, q))
        pacer.flush(("a", k))
        if k + 1 < len(turn):
            queue_halves(k + 1)
        d0, t0 = ga_at(p, q)
        w0 = 4 * 384 * (7 * (k // 7 % 3) + q)
        lhs = [ga_s.get(d0 + HB * (r - 2), d0 + HB * (r - 1), t0 + 3 * (r - 2), t0 + 3 * (r - 1)) if r in (2, 3)
               else gc_s.get(HB * (7 * (k % 2) + r), HB * (7 * (k % 2) + r + 1), 0, 3) for r in range(7)]
        rhs = [_halves(wd_s.get(w0 + 384 * (r // 2), w0 + 384 * (r // 2 + 1), r % 2)) for r in range(7)]
        last = seventh(p, q)
        out = {}
        for c in range(0, HB, ROWS):
            m = {}
            for r in ORDER1:
                m[r] = pacer.dot(_rows(lhs[r], c // 2, (c + ROWS) // 2), rhs[r], 3 * ROWS // 4)
                for i, n in _TERMS:
                    if r == _last(i, n):
                        v = _out4(m.get, i, n, ORDER1[::-1]) + last(HB * i + c, ROWS, n)
                        out.setdefault((i, n), []).append(v)
                for _ in range(0 if c else {1: 1, 2: 1, 5: 2}.get(r, 0)):
                    next(extra, None)
        return {c: _cat(v, 0) for c, v in out.items()}

    def inner(p, m):
        low[p] = {c: [[_out4(lambda q: m[q][c], i, j, ORDER1) for j in range(2)] for i in range(2)] for c in m[0]}

    def sevenths(p, m):
        for q in ORDER1:
            last = seventh(p, q)
            for i, n in m[q]:
                m[q][i, n] += last(HB * i, HB, n)
                yield
        inner(p, m)

    def queue_finish(hi, hj):
        have = [p for p in ORDER1 if p in low and p in _TERMS[hi, hj]]
        for i3, n in low[have[0]]:
            def emit(marks, i3=i3, n=n):
                def term(p):
                    v = _cat([_cat([_rows(w, QB * b, QB * (b + 1)) for w in low[p][i3, n][i]], 1)
                              for b in range(2) for i in range(2)], 0)
                    return pacer.tie(v, marks) if p == have[-1] else v
                o = _out4(term, hi, hj, have) * scale + _tile(b2, 4 * n + 2 * hj, 2)
                for b in range(2):
                    r0, c0 = (2 * i3 + b) * TB + HB * hi, 512 * n + 256 * hj
                    v = _rows(o, HB * b, HB * (b + 1)) + x_s[r0:r0 + HB, c0:c0 + 256].astype(F32)
                    if len(have) == len(_TERMS[hi, hj]):
                        x_s[r0:r0 + HB, c0:c0 + 256] = v.astype(BF)
                    else:
                        partial[i3, n, b] = v
            pacer.collect("f", GAP["finish_last" if len(low) == 6 else "finish"], ("f", hi, hj), 2 * HB // 16, emit)

    def send_block(hi, hj):
        for blk in range(NB):
            for n in range(2):
                send(blk * TB + HB * hi, HB, 512 * n + 256 * hj, 256)

    def send_last(m, blocks):
        wins = []
        for i, j in blocks:
            for i3, n in m[ORDER1[0]]:
                v = _out4(lambda q: m[q][i3, n], i, j, ORDER1[::-1])
                for b in range(2):
                    r0, c0 = (2 * i3 + b) * TB + QB * i, 512 * n + 128 * j
                    rest = lax.slice(partial[i3, n, b], (QB * i, 128 * j), (QB * (i + 1), 128 * (j + 1)))
                    x_s[r0:r0 + QB, c0:c0 + 128] = (_rows(v, QB * b, QB * (b + 1)) * scale + rest).astype(BF)
                    wins.append((r0, QB, c0, 128))
        for win in wins:
            send(*win)

    pacer.flush(("w2", 0))
    first = {}
    for q in ORDER1:
        if q == ORDER1[-1]:
            queue_halves(7)
        first[q] = two_levels(ORDER1[0], q)
    pacer.flush(("g", NP - 1))
    for k in range(1, 7):
        p = ORDER1[k]
        pacer.flush(("w2", k))
        if k == 2:
            split()
        if k == 6:
            pacer.flush(("f", 1, 0))
            pacer.flush(("f", 0, 1))
            send_block(1, 0)
            send_block(0, 1)
            split()
        else:
            queue_w2(k + 1)
        for c in {2: [(1, 0)], 4: [(0, 1)], 6: [(1, 1), (0, 0)]}.get(k, ()):
            queue_finish(*c)
        late = sevenths(ORDER1[0], first) if k == 1 else iter(())
        m = {}
        for q in ORDER1:
            if k == 6 and q == ORDER1[4]:
                pacer.flush(("f", 1, 1))
                pacer.flush(("f", 0, 0))
                send_last(m, [(1, 0), (0, 1)])
                send_block(1, 1)
            if k == 6 and q == ORDER1[6]:
                send_last(m, [(1, 1)])
            m[q] = three_levels(p, q, late)
        next(late, None)
        if k < 6:
            inner(p, m)
    send_last(m, [(0, 0)])
    for c in copies:
        c.wait()


@jax.jit
def pallas_sequential_preLN__sliding_block__mixer_channel_mlp__prompt_kernel(
        A_x, A_wqkv, A_wo, B_x, B_w1, B_b1, B_w2, B_b2):
    del B_x
    any_spec = pl.BlockSpec(memory_space=pl.ANY)
    out = pl.pallas_call(
        _kernel,
        out_shape=jax.ShapeDtypeStruct((S, D), BF),
        in_specs=[any_spec] * 7,
        out_specs=any_spec,
        scratch_shapes=[
            pltpu.VMEM((S, D), BF), pltpu.VMEM((D, D), BF), pltpu.VMEM((D, F), BF), pltpu.VMEM((F, D), BF),
            pltpu.VMEM((F,), BF), pltpu.VMEM((D,), BF),
            pltpu.VMEM((2 * TB, D), F32), pltpu.VMEM((512, 512), F32),
            pltpu.VMEM((3 * W, 256), I32), pltpu.VMEM((49 * S // 8, 256), I32),
            pltpu.VMEM((49 * 128 * 4, 256), I32), pltpu.VMEM((48384, 256), I32),
            pltpu.SemaphoreType.DMA((19,)), pltpu.SemaphoreType.DMA((14 * NB,)),
        ],
        compiler_params=pltpu.CompilerParams(vmem_limit_bytes=127 << 20),
        name="fused_block",
    )(A_x.reshape(S, D), A_wqkv, A_wo, B_w1, B_b1, B_w2, B_b2)
    return out.reshape(1, S, D)
```

```python
import math

import jax
import jax.numpy as jnp
from jax import lax
import jax.experimental.pallas as pl
import jax.experimental.pallas.tpu as pltpu

S, D, F = 2048, 1024, 3584
DH, W = 32, 256
EPS = 1e-5
TB = 512
NB = S // TB
HB, QB = TB // 2, TB // 4
NP = F // 512
BF, F32, I32 = jnp.bfloat16, jnp.float32, jnp.int32

GS = (math.sqrt(2.0 / math.pi) * 0.044715) ** (1.0 / 3.0)
GK = math.sqrt(2.0 / math.pi) / GS

GAP = {
    "exp": 25, "o": 150, "x": (None, 116, 410, 410), "h": (130, 113, 113, 113),
    "wa": {(0, 0): 27, (0, 1): 31, (0, 2): 31, (1, 0): 50, (1, 1): 83, (1, 2): 135},
    "wo": 225, "w1": (45, 45, 19, 19, 108, 108, 108), "w2": (66, 66, 69.5) + (60.5,) * 4,
    "gelu": (48,) * (NP - 1) + (41.5,), "halves": 32, "finish": 150, "finish_last": 24,
}
COST = {"exp": 9, "o": 9, "xc": 9, "hc": 1, "w": 9, "g": 14, "a": 7, "f": 9}
COST_FIRST = {"xc": 24, "hc": 1, "w": 24}
W1_WHEN = {"wo": (0, 1), 0: (2, 3), 1: (4,), 2: (5,), 3: (6,)}
ROWS = 64
TRANSPOSE_TIME = 900
REDUCE_TIME = 180
NORM_TIME = 200
SCORE_PACE = 0.8
EARLY = ((2, 4), (3, 6))


def _cat(xs, axis):
    return xs[0] if len(xs) == 1 else lax.concatenate(xs, axis)


def _rows(x, r0, r1):
    return lax.slice_in_dim(x, r0, r1, axis=0)


def _tile(x, t, n=1):
    return lax.slice_in_dim(x, 128 * t, 128 * (t + n), axis=1)


def _words(x):
    return pltpu.bitcast(x.astype(BF), I32)


def _halves(w):
    return pltpu.bitcast(w, BF) if w.dtype == I32 else w


def _dot(a, b):
    return lax.dot_general(_halves(a), _halves(b), (((1,), (0,)), ((), ())), preferred_element_type=F32)


def _dot_nt(a, b):
    return lax.dot_general(_halves(a), _halves(b), (((1,), (1,)), ((), ())), preferred_element_type=F32)


def _layernorm(x, scales=None):
    m = jnp.mean(x, axis=-1, keepdims=True)
    yield
    xc = x - m
    v = jnp.mean(xc * xc, axis=-1, keepdims=True)
    yield
    r = lax.rsqrt(v + EPS)
    if scales is None:
        return xc * r
    n = x.shape[1] // 128 // len(scales)
    rs = {c: r * c for c in scales}
    return _cat([_tile(xc, n * i, n) * rs[c] for i, c in enumerate(scales)], 1)


def _lhs7(a):
    (a11, a12), (a21, a22) = a
    return [a11 + a22, a21 + a22, a11, a22, a11 + a12, a21 - a11, a12 - a22]


def _rhs7(b):
    (b11, b12), (b21, b22) = b
    return [b11 + b22, b11, b12 - b22, b21 - b11, b22, b11 + b12, b21 + b22]


_TERMS = {(0, 0): {0: 1, 3: 1, 4: -1, 6: 1}, (0, 1): {2: 1, 4: 1},
          (1, 0): {1: 1, 3: 1}, (1, 1): {0: 1, 1: -1, 2: 1, 5: 1}}
ORDER1 = (1, 3, 2, 4, 5, 0, 6)
ORDER2 = (ORDER1, (6, 1, 3, 2, 4, 5, 0))


def _out4(m, i, j, order):
    acc = None
    for p in reversed(order):
        sign = _TERMS[i, j].get(p)
        if sign and acc is None:
            acc = m(p) if sign > 0 else -m(p)
        elif sign:
            acc = acc + m(p) if sign > 0 else acc - m(p)
    return acc


def _last(i, j):
    return [p for p in ORDER1 if p in _TERMS[i, j]][-1]


_ROW = (1.0, math.sqrt(3.0), math.sqrt(3.0), 3.0)
_COL = _ROW[::-1]
BAL1 = (0, 1, 2, 4, 6, 3, 5)
BAL2 = ((1, 2, 4, 6, 3, 5, 0), BAL1)


def _bal_lhs7(a):
    (a11, a12), (a21, a22) = a
    s, t = a11 + a22, a12 + a21
    return [s, a11 - a12, a11 + a12, s - t, a12 - a22, s + t, a12 + a22]


def _bal_rhs7(b):
    (b11, b12), (b21, b22) = b
    s, t = b11 + b22, b12 + b21
    return [s + s, b12 - b22, b12 + b22, b11 + b12, s + t, b11 - b12, s - t]


def _bal_out(m, order):
    c12, e = m[1] + m[2], m[1] - m[2]
    c21 = (c12 - (m[4] + m[6])) + (m[5] - m[3])
    if order[0] == 0:
        d = e + m[0]
        return [[d + (m[4] - m[6]), c12], [c21, d - (m[3] + m[5])]]
    return [[(e + (m[4] - m[6])) + m[0], c12], [c21, (e - (m[3] + m[5])) + m[0]]]


STD_TURN = (ORDER1, ((0, 0), (1, 1)))
BAL_TURN = ((1, 2, 3, 5, 0, 4, 6), ((0, 0), (0, 1)))


def _nested(f, a, hold=lambda q, k, v: v):
    low = {(hi, hj): f([[a[2 * hi + i][2 * hj + j] for j in range(2)] for i in range(2)])
           for hi in range(2) for hj in range(2)}
    return {(p, q): v for q in range(7)
            for p, v in enumerate(f([[hold(q, (hi, hj), low[hi, hj][q]) for hj in range(2)] for hi in range(2)]))}


def _lane_bits(shape):
    lane = lax.broadcasted_iota(I32, shape, 1)
    return (lane & 32) == 0, (lane & 64) == 0


def _butterfly(v, b0, b1):
    u = [lax.select(b0, v[i], v[i ^ 1]) for i in range(4)]
    return [lax.select(b1, u[i], u[i ^ 2]) for i in range(4)]


class _Pacer:
    def __init__(self):
        self.masks = {}
        self.now = 0.0
        self.mark = None
        self.busy = 0.0
        self.free = {}
        self.events = []
        self.dues = []

    def tie(self, value, marks):
        known = [m for m in marks if m is not None]
        if not known:
            return value
        if value.shape not in self.masks:
            lane = lax.broadcasted_iota(I32, value.shape, 1) & 127
            self.masks[value.shape] = lane * lane == 2
        n = value.shape[0] // 8 // len(marks)
        wait = _cat([known[-1] if m is None else m for m in marks for _ in range(n)], 0)
        if wait.dtype != value.dtype:
            wait = pltpu.bitcast(wait, value.dtype)
        return lax.select(self.masks[value.shape], _cat([wait] * (value.shape[1] // 128), 1), value)

    def due(self, value, delay):
        self.dues.append((self.now + delay, pltpu.bitcast(value, I32)))

    def at(self, t, tag, job):
        self.events.append((t, tag, job))
        self.events.sort(key=lambda e: e[0])

    def add(self, lane, gap, tag, job, delay=0):
        t = max(self.now + delay, self.free.get(lane, 0.0))
        self.free[lane] = t + gap
        self.at(t, tag, job)

    def collect(self, lane, gap, tag, n, then, delay=0, group=0):
        marks = []

        def job():
            marks.append(self.mark)
            if len(marks) == n:
                then(marks)
            return COST_FIRST[lane] if group and len(marks) % group == 1 else COST[lane]
        for _ in range(n):
            self.add(lane, gap, tag, job, delay)

    def stepwise(self, tag, steps):
        def job():
            if next(steps, self) is not self:
                self.at(self.now + REDUCE_TIME, tag, job)
            return 1
        return job

    def tick(self, r, cycles):
        n = r.shape[0] // 8
        for i in range(n):
            self.now += cycles / n
            if self.events and max(self.busy, self.events[0][0]) <= self.now:
                self.mark = lax.slice(r, (8 * i, 0), (8 * i + 8, 128))
                self.busy = self.now + self.events.pop(0)[2]()
        self.mark = None

    def flush(self, tag):
        while tag in [e[1] for e in self.events]:
            t, _, job = self.events.pop([e[1] for e in self.events].index(tag))
            self.now, now = t, self.now
            job()
            self.now = now

    def dot(self, lhs, rhs, cycles, last=True):
        n = lhs.shape[0]
        for t, v in self.dues:
            if t < self.now + cycles:
                i = 8 * max(0, int((t - self.now) * (n // 8) / cycles))
                parts = [_rows(lhs, 0, i)] if i else []
                parts.append(self.tie(_rows(lhs, i, i + 8), [v]))
                lhs = _cat(parts + ([_rows(lhs, i + 8, n)] if i + 8 < n else []), 0)
        r = _dot(lhs, rhs)
        if last:
            self.dues = [d for d in self.dues if d[0] >= self.now + cycles]
            self.tick(r, cycles)
        return r


class _Words:
    def __init__(self, pool, start, rows, tiles):
        self.pool, self.start, self.rows = pool, start, rows // 2
        self.end = start + self.rows * ((tiles + 1) // 2)
        assert self.end <= pool.shape[0]

    def _window(self, r0, n, t, k):
        r = self.start + (t // 2) * self.rows + r0 // 2
        return slice(r, r + n), slice(128 * (t % 2), 128 * (t % 2 + k))

    def _runs(self, t0, t1):
        while t0 < t1:
            k = 2 if t0 % 2 == 0 and t0 + 1 < t1 else 1
            yield t0, k
            t0 += k

    def get(self, r0, r1, t0, t1=None):
        return _cat([self.pool[self._window(r0, (r1 - r0) // 2, t, k)] for t, k in self._runs(t0, t1 or t0 + 1)], 1)

    def put(self, r0, t0, x):
        runs = list(self._runs(t0, t0 + x.shape[1] // 128))
        for t, k in runs:
            part = x if len(runs) == 1 else _tile(x, t - t0, k)
            self.pool[self._window(r0, x.shape[0] // 2, t, k)] = _words(part)


def _interleave(a, na, b, nb):
    ia = ib = 0
    while ia < na or ib < nb:
        if ib >= nb or (ia < na and ia * nb <= ib * na):
            next(a)
            ia += 1
        else:
            next(b)
            ib += 1


def _kernel(x_hbm, wqkv_hbm, wo_hbm, w1_hbm, b1_hbm, w2_hbm, b2_hbm, o_hbm,
            x_s, wo_s, w1_s, w2_s, b1_s, b2_s, y_s, o_s, p_pool, ya_pool, wb_pool, pool, sem_in, sem_out):
    pacer = _Pacer()
    sems = iter(range(sem_in.shape[0]))

    def copy(src, dst):
        return pltpu.make_async_copy(src, dst, sem_in.at[next(sems)])

    def wqkv_copy(m, c0, n):
        return copy(wqkv_hbm.at[:, pl.ds(m * D + c0, n)], w2_s.at[pl.ds(m * D, D), pl.ds(c0, n)])

    def row_copy(src, dst, r0, r1):
        return copy(src.at[pl.ds(r0, r1 - r0)], dst.at[pl.ds(r0, r1 - r0)])

    first_rows = (0, HB, QB, HB + QB)
    stages = [[row_copy(x_hbm, x_s, r, r + QB)] for r in first_rows] + [
        [wqkv_copy(0, 0, 128)],
        [wqkv_copy(0, 128, 384)],
        [wqkv_copy(1, 0, 512)],
        [wqkv_copy(2, 0, 512)],
        [wqkv_copy(0, 512, 512)],
        [wqkv_copy(1, 512, 512), wqkv_copy(2, 512, 512), row_copy(x_hbm, x_s, TB, 2 * TB)],
    ]
    rest = [row_copy(x_hbm, x_s, 2 * TB, S), copy(b1_hbm, b1_s), copy(b2_hbm, b2_s), copy(wo_hbm, wo_s)]
    w1_copy = copy(w1_hbm, w1_s)
    w2_copy = copy(w2_hbm, w2_s)
    for stage in stages + [rest]:
        for c in stage:
            c.start()

    def landed():
        for c in stages.pop(0):
            c.wait()

    lane = lax.broadcasted_iota(I32, (32, 128), 1)
    row = lax.broadcasted_iota(I32, (32, 128), 0)
    top_valid = row > (lane & 31)
    lane16 = lax.broadcasted_iota(I32, (16, 128), 1)
    row16 = lax.broadcasted_iota(I32, (16, 128), 0)
    top_words = (jnp.where(2 * row16 > (lane16 & 31), 0xFFFF, 0)
                 | jnp.where(2 * row16 + 1 > (lane16 & 31), -0x10000, 0))
    low_words = ~top_words

    zero = jnp.clip((lane16 * lane16)[0, 0], 0, 1) * 8
    for buf in (y_s, o_s, p_pool, ya_pool, wb_pool, pool):
        buf[pl.ds(zero, 8), 0:128] = jnp.zeros((8, 128), buf.dtype)
    p_s = _Words(p_pool, 0, 3 * W, 4)
    xa_s = _Words(pool, 0, 2 * 49 * QB, 2)
    oa_s = _Words(pool, xa_s.end, 7 * S // 2, 4)
    q_s = _Words(pool, oa_s.end, 2 * TB, 8)
    k_s = _Words(pool, q_s.end, S, 8)
    vt_s = _Words(pool, k_s.end, D, S // 128)
    wa_s = _Words(pool, vt_s.end, 49 * 256, 6)
    xn_s = _Words(pool, wa_s.end, TB, 8)
    xb_s = _Words(pool, xn_s.end, 7 * HB, 4)
    wc_s = _Words(pool, wa_s.end, 7 * 512, 4)
    ya_s = _Words(ya_pool, 0, 49 * S // 4, 2)
    wb_s = _Words(wb_pool, 0, 49 * 256, NP)
    ga_s = _Words(pool, 0, 25 * S // 4, 2 * NP)
    gc_s = _Words(pool, ga_s.end, 14 * HB, 3)
    we_s = _Words(wb_pool, 0, 49 * 128, 2)
    wd_s = _Words(wb_pool, we_s.end, 21 * 4 * 384, 2)

    def split(wait=(), start=()):
        for c in wait:
            c.wait()
        for c in start:
            c.start()

        @pl.when(zero != 0)
        def _():
            pool[0:8, 0:128] = jnp.zeros((8, 128), I32)

    def x_rows(r0):
        x = x_s[r0:r0 + 8, :].astype(F32)
        return _cat([pacer.tie(_tile(x, 0), [pacer.mark]), _tile(x, 1, 7)], 1)

    def queue_operands(lane, gap, tag, steps, combine, turn, block, put, delay=0):
        order, held = turn

        def emit(marks):
            def hold(q, k, v):
                return pacer.tie(v, marks[order.index(q)::7]) if k in held else v
            for (p, q), v in _nested(combine, [[block(a, b) for b in range(4)] for a in range(4)], hold).items():
                put(7 * p + q, v)
        pacer.collect(lane, gap, tag, 7 * steps, emit, delay, 7)

    def queue_rows(lane, blk, group, normed, combine, turn, dest, row0):
        gap = GAP[lane][blk]
        done = []

        def steps(i, r):
            y = yield from normed(i, r)
            r0 = r // 16 * 16
            y0 = TB * (blk % 2) + r0
            y_s[y0 + QB * i + r - r0:y0 + QB * i + r - r0 + 8, :] = y
            done.append(_tile(y, 0))
            if len(done) % group == 0:
                pacer.due(sum(done[1 - group:], done[-group]), NORM_TIME)
            if len(done) % 8 == 0:
                for c in range(2):
                    queue_operands(
                        lane + "c", gap * 8 / 15, (lane, blk), 1, combine, turn,
                        lambda a, b, c=c: y_s[y0 + QB * a:y0 + QB * a + 16, 256 * b + 128 * c:256 * b + 128 * (c + 1)],
                        lambda k, v, c=c: dest.put(row0(k) + r0, c, v), NORM_TIME + 50)
        pacer.flush((lane, blk - 2))
        for r in range(0, QB, 16):
            for i in range(4):
                for rr in (r, r + 8):
                    pacer.add(lane, gap, (lane, blk), pacer.stepwise((lane, blk), steps(i, rr)))

    qscale = (DH ** -0.5) * math.log2(math.e)
    count = [0, 0]
    bits = {n: _lane_bits((n, 128)) for n in (1, 16, 32, 64, 128, 192)}
    nought = jnp.zeros((16, 128), I32)

    def queue_x(blk):
        queue_rows("x", blk, 2 if blk > 1 else 4,
                   lambda i, r: _layernorm(x_rows(blk * TB + i * QB + r), [_ROW[i] * c for c in _COL]),
                   _bal_lhs7, BAL_TURN, xa_s, lambda k: (blk % 2 * 49 + k) * QB)

    def queue_wa(j, m):
        def block(a, b):
            r0, c0 = m * D + 256 * a, 512 * j + 256 * (b // 2)
            return _tile(w2_s[r0:r0 + 256, c0:c0 + 256].astype(F32), b % 2) * (_ROW[a] * _COL[b])
        queue_operands("w", GAP["wa"][j, m], ("wa", j, m), 16, _bal_rhs7, BAL_TURN, block,
                       lambda k, v: wa_s.put(256 * k, 3 * j + m, v))

    def put_qkv(m, r0, g, c):
        if m == 0:
            q_s.put(r0 % (2 * TB), g, c)
        elif m == 1:
            k_s.put(r0, g, c)
        else:
            c = c.T
            vt_s.put(128 * g, r0 // 128, c)
        return lax.slice(c, (c.shape[0] - 8, c.shape[1] - 128), c.shape)

    def first_products(j, m):
        for g in range(4 * j, 4 * j + 4):
            if (m, g) == (0, 1):
                landed()
                queue_wa(0, 0)
            c = pacer.dot(xn_s.get(0, TB, 0, 4), w2_s[m * D:m * D + 512, 128 * g:128 * (g + 1)], TB)
            yield
            c += pacer.dot(xn_s.get(0, TB, 4, 8), w2_s[m * D + 512:(m + 1) * D, 128 * g:128 * (g + 1)], TB)
            last = put_qkv(m, 0, g, c * qscale if m == 0 else c)
            if m == 2:
                pacer.due(last, TRANSPOSE_TIME)
            yield

    def first_one_level(m):
        for g in (0, 2):
            w = w2_s[m * D:(m + 1) * D, 128 * g:128 * (g + 2)].astype(F32)
            rhs = _rhs7([[_tile(_rows(w, 512 * a, 512 * (a + 1)), b) for b in range(2)] for a in range(2)])
            prod = {}
            for p in ORDER1:
                prod[p] = pacer.dot(xb_s.get(HB * p, HB * (p + 1), 0, 4), rhs[p].astype(BF), HB)
                for i, b in _TERMS:
                    if p == _last(i, b):
                        last = put_qkv(m, HB * i, g + b, _out4(prod.get, i, b, ORDER1))
                        if m == 2:
                            pacer.due(last, TRANSPOSE_TIME)

    def qkv_products(blk, j):
        for m in range(3):
            pacer.flush(("wa", j, m))
            low = {}
            for p in BAL1:
                order = BAL2[count[0] % 2]
                count[0] += 1
                prod = {}
                for q in order:
                    k = 7 * p + q
                    o = (blk % 2 * 49 + k) * QB
                    prod[q] = pacer.dot(xa_s.get(o, o + QB, 0, 2), wa_s.get(256 * k, 256 * (k + 1), 3 * j + m),
                                        QB * (876 - 288 * SCORE_PACE) / 588, count[1] % 2)
                    count[1] += 1
                    if q == order[-1]:
                        low[p] = _bal_out(prod, order)
                        if p == BAL1[-1]:
                            finish_qkv(blk, j, m, low)
                    if count[1] % 2 == 0:
                        yield

    def finish_qkv(blk, j, m, low):
        c = {}
        for i in range(2):
            for k in range(2):
                t = _bal_out({p: low[p][i][k] for p in BAL1}, BAL1)
                c.update({(2 * hi + i, 2 * hj + k): t[hi][hj] for hi in range(2) for hj in range(2)})
        turn = ((0, 1), (0, 0), (1, 0), (1, 1))
        for hi, hj in turn:
            for i, k in turn:
                a, b = 2 * hi + i, 2 * hj + k
                scale = (qscale if m == 0 else 1.0) / (12 * _ROW[a] * _COL[b])
                last = put_qkv(m, blk * TB + a * QB, 4 * j + b, c[a, b] * scale)
        if m == 2:
            pacer.due(last, TRANSPOSE_TIME)

    def scores(sb, g, slot, turn=(0, 1, 2, 3)):
        j0 = max(0, 8 - 4 * sb)
        ss, ms = {}, {}
        b0, b1 = bits[16]
        for t in turn:
            qt = q_s.get(128 * (sb % 8) + 32 * t, 128 * (sb % 8) + 32 * (t + 1), g)
            q2 = [lax.select(b0, qt, nought), lax.select(b0, nought, qt)]
            q4 = [lax.select(b1, v, nought) for v in q2] + [lax.select(b1, nought, v) for v in q2]
            lo = max(j0, t)
            keys = k_s.get(128 * sb - W + 32 * lo, 128 * sb - W + 32 * (t + 9), g)
            s = _dot_nt(keys, _cat([q4[c ^ t] for c in range(4)], 0))
            n = s.shape[0]
            if t == 3:
                pacer.tick(s, n * SCORE_PACE)
            first = _rows(s, 0, 32) if lo == t else jnp.full((32, 128), -jnp.inf, F32)
            body = [_rows(s, 32 if lo == t else 0, n - 32)] if n > 32 else []
            ss[t] = _cat(body + [lax.select(top_valid, first, _rows(s, n - 32, n))], 0)
            ms[t] = jnp.broadcast_to(jnp.max(ss[t], axis=0, keepdims=True), (8, 128))
        todo = [(j, t) for j in range(j0, 12) for t in range(4) if 0 <= j - t < 8 or (j - t == 8 and t < j0)]
        sums = []

        def emit(marks):
            ends = [ss[t].shape[0] - (0 if j == t else 32 * (8 + t - j)) for j, t in todo]
            s = _cat([_rows(ss[t], e - 32, e) for (_, t), e in zip(todo, ends)], 0)
            p = jnp.exp2(s - pacer.tie(_cat([ms[t] for _, t in todo for _ in range(4)], 0), marks))
            for t in range(4):
                pt = _cat([_rows(p, 32 * k, 32 * (k + 1)) for k, (_, u) in enumerate(todo) if u == t], 0)
                sums.append(jnp.sum(pt, axis=0, keepdims=True))
                p_s.put(W * slot, t, pt)
        pacer.collect("exp", GAP["exp"], (sb, g), len(todo), emit)
        return sums

    def values(sb, g, slot, sums):
        j0 = max(0, 8 - 4 * sb)
        pacer.flush((sb, g))
        inv = _butterfly([pltpu.reciprocal(l, full_range=False) for l in sums], *bits[1])
        v = []
        for t in range(4):
            n = min(8, 9 + t - j0)
            w = p_s.get(W * slot, W * slot + 32 * n, t)
            parts = [w]
            if t >= j0:
                edge = _rows(w, 0, 16)
                parts = [nought] * (t - j0) + [edge & top_words, _rows(w, 16, 16 * n), edge & low_words]
            v.append(_cat(parts + [nought] * (3 - t), 0))
        heads = _butterfly(v, *bits[v[0].shape[0]])
        outs = [None] * 4
        for k in range(3 - j0 // 4):
            for h in range(4):
                vt = vt_s.get(128 * g + DH * h, 128 * g + DH * (h + 1), sb - 2 + j0 // 4 + k)
                o = _dot(vt, _rows(heads[h], 64 * k, 64 * (k + 1)))
                outs[h] = o if k == 0 else outs[h] + o
        ot = _cat([o * i for o, i in zip(outs, inv)], 0).T
        pacer.due(_rows(ot, 120, 128), TRANSPOSE_TIME)
        r0, c0 = 256 * (sb % 2), 256 * (g // 2 % 2)
        pacer.flush(("o", r0, c0))
        a0, b0 = r0 + 128 * (sb % 4 // 2), c0 + 128 * (g % 2)
        o_s[a0:a0 + 128, b0:b0 + 128] = _cat(_butterfly([_rows(ot, r, r + 32) for r in range(0, 128, 32)], *bits[32]), 0)
        if sb % 4 >= 2 and g % 2:
            def emit(marks):
                a = [[o_s[r0 + 128 * i:r0 + 128 * (i + 1), c0 + 128 * b:c0 + 128 * (b + 1)] for b in range(2)]
                     for i in range(2)]
                for i in range(2):
                    a[i][i] = pacer.tie(a[i][i], marks)
                for p, v in enumerate(_lhs7(a)):
                    oa_s.put(((sb // 4) * 7 + p) * HB + 128 * (sb % 2), g // 2, v)
            pacer.collect("o", GAP["o"], ("o", r0, c0), 8, emit, TRANSPOSE_TIME + 50)

    def attention():
        units = [(4 * blk + s, 4 * j + g + b) for blk in range(NB) for j in range(2) for g in (2, 0)
                 for s in (0, 2, 1, 3) for b in range(2)]
        prev = None
        for n, u in enumerate(units):
            if u[0] >= 2:
                sums = scores(*u, n % 3)
            elif n % 2 == 0:
                sums = scores(*u, n % 3)
                ahead = scores(*units[n + 1], (n + 1) % 3, (3, 2, 1, 0))
            else:
                sums = ahead
            yield
            if prev:
                values(*prev)
            prev = (*u, n % 3, sums)
            yield
        yield
        values(*prev)
        yield

    def queue_wo(n):
        def emit(marks):
            def block(a, b):
                w = _cat([wo_s[128 * k:128 * (k + 1), 256 * n:256 * (n + 1)] for k in range(a, 8, 2)], 0)
                w = _tile(w.astype(F32), b)
                return pacer.tie(w, marks) if a == b else w
            for p, v in enumerate(_rhs7([[block(a, b) for b in range(2)] for a in range(2)])):
                wc_s.put(512 * p, n, v)
        pacer.collect("w", GAP["wo"], "wo", 32, emit)

    def wo_products(blk):
        c = {}
        for n in range(4):
            prod = {}
            for p in ORDER1:
                o = (blk * 7 + p) * HB
                prod[p] = pacer.dot(oa_s.get(o, o + HB, 0, 4), wc_s.get(512 * p, 512 * (p + 1), n), HB)
                if p == ORDER1[-1]:
                    for i in range(2):
                        for b in range(2):
                            c[i, 2 * n + b] = _out4(prod.get, i, b, ORDER1)
                    if n == 3:
                        queue_h(blk, _cat([_cat([c[i, t] for t in range(8)], 1) for i in range(2)], 0))
                yield

    def queue_h(blk, o):
        hs = {}

        def normed(i, r):
            r0 = blk * TB + i * QB + r
            h = hs[i, r] = x_rows(r0) + _rows(o, i * QB + r, i * QB + r + 8)
            if r % 16:
                x_s[r0 - 8:r0 + 8, :] = _cat([hs[i, r - 8], h], 0).astype(BF)
            return (yield from _layernorm((yield from _layernorm(h)), (GS,)))
        queue_rows("h", blk, 4, normed, _lhs7, STD_TURN, ya_s, lambda k: k * (S // 4) + blk * QB)

    def queue_w1(n):
        def block(a, b):
            c0 = 512 * n + 256 * (b // 2)
            return _tile(w1_s[256 * a:256 * (a + 1), c0:c0 + 256].astype(F32), b % 2)
        queue_operands("w", GAP["w1"][n], ("w1", n), 16, _rhs7, STD_TURN, block,
                       lambda k, v: wb_s.put(256 * k, n, v))

    ga = attention()
    xn = {}
    for r in first_rows:
        landed()

        def steps(r=r):
            xn[r] = yield from _layernorm(x_s[r:r + QB, :].astype(F32))
        list(steps())
        xn_s.put(r, 0, xn[r])
        if r >= HB:
            for p, v in enumerate(_lhs7([[_tile(xn[i], 4 * k, 4) for k in range(2)] for i in (r - HB, r)])):
                xb_s.put(HB * p + r - HB, 0, v)
    landed()
    list(first_products(0, 0))
    landed()
    queue_wa(0, 1)
    first_one_level(1)
    landed()
    queue_wa(0, 2)
    first_one_level(2)
    landed()
    queue_wa(1, 0)
    _interleave(first_products(1, 0), 8, ga, 17)
    landed()
    queue_x(1)
    queue_wa(1, 1)
    _interleave((None for m in (1, 2) for _ in first_products(1, m)), 16, ga, 14)
    for blk in range(1, NB):
        pacer.flush(("x", blk))
        if blk == 1:
            queue_wa(1, 2)
            split(wait=rest, start=[w1_copy])
        if blk < NB - 1:
            queue_x(blk + 1)
        else:
            for n in range(4):
                queue_wo(n)
        for j in range(2):
            gp = qkv_products(blk, j)
            _interleave(gp, (147 + count[1] % 2) // 2, ga, 32)
            next(gp, None)
    pacer.flush("wo")
    split(wait=[w1_copy], start=[w2_copy])
    for n in W1_WHEN["wo"]:
        queue_w1(n)
    _interleave(wo_products(0), 28, ga, 17)
    _interleave(wo_products(1), 28, ga, 18)
    list(wo_products(2))
    for r0 in (0, 256):
        for c0 in (0, 256):
            pacer.flush(("o", r0, c0))
    list(wo_products(3))

    b1 = b1_s[...].astype(F32).reshape(1, F) * GS
    b2 = b2_s[...].astype(F32).reshape(1, D)

    def ga_at(p, q):
        k = 7 * p + q
        return k // 2 * (S // 4), k % 2 * NP

    def queue_gelu(n, low):
        keys = [(i, j, hj) for i, j in ((0, 1), (1, 0), (0, 0), (1, 1)) for hj in range(2)]

        def emit(marks):
            zs = []
            for k, (i, j, hj) in enumerate(keys):
                m = {p: low[p][i][j] for p in ORDER1}
                both = 3 - hj
                bias = jnp.broadcast_to(_tile(b1, 4 * n + 2 * hj + j), (S // 4, 128))
                m[both] = m[both] + pacer.tie(bias, marks[k::8])
                zs += [_out4(m.get, hi, hj, [p for p in ORDER1 if p != both] + [both]) for hi in range(2)]
            z = _cat([_rows(v, r, r + 16) for r in range(0, S // 4, 16) for v in zs], 0)
            g = z * jnp.tanh(z * (z * z + GK)) + z
            a = [[None] * 4 for _ in range(4)]
            for k, (i, j, hj) in enumerate(keys):
                for hi in range(2):
                    a[2 * hi + i][2 * hj + j] = _cat([_rows(g, 16 * (r + 2 * k + hi), 16 * (r + 2 * k + hi + 1))
                                                      for r in range(0, S // 4, 16)], 0)
            for (p, q), v in _nested(_lhs7, a).items():
                d0, t0 = ga_at(p, q)
                ga_s.put(d0, t0 + n, v)
        pacer.collect("g", GAP["gelu"][n], ("g", n), 8 * S // 64, emit)

    def queue_w2(k):
        p = ORDER1[k]

        def inner(positions, n):
            def block(a, b):
                c0 = 512 * n + 256 * (b // 2)
                w = [w2_s[512 * t + 128 * a:512 * t + 128 * (a + 1), c0:c0 + 256].astype(F32) for t in positions]
                return _tile(_cat(w, 0), b % 2)
            return _rhs7([[_rhs7([[block(2 * hi + i, 2 * hj + j) for hj in range(2)] for hi in range(2)])[p]
                           for j in range(2)] for i in range(2)])

        def emit(marks):
            low = [[inner(range(3 * i, 3 * i + 3), n) for n in range(2)] for i in range(2)]
            for q in range(7):
                v = [[low[i][n][q] for n in range(2)] for i in range(2)]
                for i in range(2):
                    for n in (i,) if k else range(2):
                        v[i][n] = pacer.tie(v[i][n], marks[ORDER1.index(q)::7])
                for r, w in enumerate(_rhs7(v) if k else v[0] + v[1]):
                    wd_s.put(384 * (4 * (7 * (k % 3) + q) + r // 2), r % 2, w)

        def emit_seventh(marks):
            for n in range(2):
                for q, w in enumerate(inner([NP - 1], n)):
                    we_s.put(128 * (7 * p + q), n, pacer.tie(w, marks[n::2]))
        pacer.collect("w", GAP["w2"][k], ("w2", k), 16, emit_seventh)
        pacer.collect("w", GAP["w2"][k], ("w2", k), 7 * 24, emit, 0, 7)

    def w1_products(n, p, b0, b1):
        order = ORDER2[count[0] % 2]
        count[0] += 1
        m = {}
        for q in order:
            k = 7 * p + q
            rhs = wb_s.get(256 * k, 256 * (k + 1), n)
            r0, r1 = k * (S // 4) + b0 * QB, k * (S // 4) + b1 * QB
            if (p, q, b1) == (ORDER1[-1], order[-1], NB):
                rm = (r0 + r1) // 2
                m[q] = _cat([pacer.dot(ya_s.get(r0, rm, 0, 2), rhs, rm - r0, False),
                             pacer.dot(ya_s.get(rm, r1, 0, 2), rhs, rm - r0)], 0)
            else:
                m[q] = pacer.dot(ya_s.get(r0, r1, 0, 2), rhs, r1 - r0, count[1] % 2)
            count[1] += 1
        return m, order

    low = None
    for n in range(NP):
        pacer.flush(("w1", n))
        if n == 3:
            pacer.flush(("g", n - 2))
            split(wait=[w2_copy])
        if n:
            queue_gelu(n - 1, low)
        if n >= NP - 2:
            queue_w2(n - NP + 2)
        count[:] = [0, 0]
        done = {p: (0, []) for p in ORDER1}
        if n == 0:
            for upto, some in EARLY:
                for b in range(upto):
                    pacer.flush(("h", b))
                for p in ORDER1[:some]:
                    done[p] = (upto, done[p][1] + [w1_products(n, p, done[p][0], upto)[0]])
            pacer.flush(("h", NB - 1))
            pacer.dues = []
        for k in W1_WHEN.get(n, ()):
            queue_w1(k)
        low = {}
        for p in ORDER1:
            tail, order = w1_products(n, p, done[p][0], NB)
            m = {q: _cat([v[q] for v in done[p][1] + [tail]], 0) for q in order}
            low[p] = [[_out4(m.get, i, j, order) for j in range(2)] for i in range(2)]
    for n in range(NP - 1):
        pacer.flush(("g", n))
    queue_gelu(NP - 1, low)

    turn = [(p, q) for p in ORDER1 for q in ORDER1]
    scale = 0.5 / GS
    low, partial, copies = {}, {}, []

    def send(r0, rows, c0, cols):
        win = (pl.ds(r0, rows), pl.ds(c0, cols))
        copies.append(pltpu.make_async_copy(x_s.at[win], o_hbm.at[win], sem_out.at[len(copies)]))
        copies[-1].start()

    def queue_halves(k):
        d0, t0 = ga_at(*turn[k])

        def emit(marks):
            def block(i, j):
                w = [ga_s.get(d0 + HB * i, d0 + HB * (i + 1), t0 + 3 * j + t) for t in range(3)]
                w = [pacer.tie(w[t], marks[t::3]) if i == j else w[t] for t in range(3)]
                return _halves(_cat(w, 1)).astype(F32)
            for r, v in enumerate(_lhs7([[block(i, j) for j in range(2)] for i in range(2)])):
                if r not in (2, 3):
                    gc_s.put(HB * (7 * (k % 2) + r), 0, v)
        pacer.collect("a", GAP["halves"], ("a", k), 3 * HB // 16, emit)

    def seventh(p, q):
        d0, t0 = ga_at(p, q)
        lhs = ga_s.get(d0, d0 + S // 4, t0 + NP - 1)
        rhs = [_halves(we_s.get(128 * (7 * p + q), 128 * (7 * p + q + 1), n)) for n in range(2)]

        def product(r0, rows, n):
            pacer.now += rows // 4
            return _dot(_rows(lhs, r0 // 2, (r0 + rows) // 2), rhs[n])
        return product

    def two_levels(p, q):
        d0, t0 = ga_at(p, q)
        w0 = 4 * 384 * q
        out = {}
        for i in range(2):
            rows = (d0 + HB * i, d0 + HB * (i + 1))
            c = pacer.dot(ga_s.get(*rows, t0 + 4, t0 + 6), wd_s.get(w0 + 512, w0 + 768, 0, 2), HB)
            for n in range(2):
                out[i, n] = _tile(c, n) + pacer.dot(ga_s.get(*rows, t0, t0 + 4), wd_s.get(w0, w0 + 512, n), HB)
        return out

    def three_levels(p, q, extra):
        k = turn.index((p, q))
        pacer.flush(("a", k))
        if k + 1 < len(turn):
            queue_halves(k + 1)
        d0, t0 = ga_at(p, q)
        w0 = 4 * 384 * (7 * (k // 7 % 3) + q)
        lhs = [ga_s.get(d0 + HB * (r - 2), d0 + HB * (r - 1), t0 + 3 * (r - 2), t0 + 3 * (r - 1)) if r in (2, 3)
               else gc_s.get(HB * (7 * (k % 2) + r), HB * (7 * (k % 2) + r + 1), 0, 3) for r in range(7)]
        rhs = [_halves(wd_s.get(w0 + 384 * (r // 2), w0 + 384 * (r // 2 + 1), r % 2)) for r in range(7)]
        last = seventh(p, q)
        out = {}
        for c in range(0, HB, ROWS):
            m = {}
            for r in ORDER1:
                m[r] = pacer.dot(_rows(lhs[r], c // 2, (c + ROWS) // 2), rhs[r], 3 * ROWS // 4)
                for i, n in _TERMS:
                    if r == _last(i, n):
                        v = _out4(m.get, i, n, ORDER1[::-1]) + last(HB * i + c, ROWS, n)
                        out.setdefault((i, n), []).append(v)
                for _ in range(0 if c else {1: 1, 2: 1, 5: 2}.get(r, 0)):
                    next(extra, None)
        return {c: _cat(v, 0) for c, v in out.items()}

    def inner(p, m):
        low[p] = {c: [[_out4(lambda q: m[q][c], i, j, ORDER1) for j in range(2)] for i in range(2)] for c in m[0]}

    def sevenths(p, m):
        for q in ORDER1:
            last = seventh(p, q)
            for i, n in m[q]:
                m[q][i, n] += last(HB * i, HB, n)
                yield
        inner(p, m)

    def queue_finish(hi, hj):
        have = [p for p in ORDER1 if p in low and p in _TERMS[hi, hj]]
        for i3, n in low[have[0]]:
            def emit(marks, i3=i3, n=n):
                def term(p):
                    v = _cat([_cat([_rows(w, QB * b, QB * (b + 1)) for w in low[p][i3, n][i]], 1)
                              for b in range(2) for i in range(2)], 0)
                    return pacer.tie(v, marks) if p == have[-1] else v
                o = _out4(term, hi, hj, have) * scale + _tile(b2, 4 * n + 2 * hj, 2)
                for b in range(2):
                    r0, c0 = (2 * i3 + b) * TB + HB * hi, 512 * n + 256 * hj
                    v = _rows(o, HB * b, HB * (b + 1)) + x_s[r0:r0 + HB, c0:c0 + 256].astype(F32)
                    if len(have) == len(_TERMS[hi, hj]):
                        x_s[r0:r0 + HB, c0:c0 + 256] = v.astype(BF)
                    else:
                        partial[i3, n, b] = v
            pacer.collect("f", GAP["finish_last" if len(low) == 6 else "finish"], ("f", hi, hj), 2 * HB // 16, emit)

    def send_block(hi, hj):
        for blk in range(NB):
            for n in range(2):
                send(blk * TB + HB * hi, HB, 512 * n + 256 * hj, 256)

    def send_last(m, blocks):
        wins = []
        for i, j in blocks:
            for i3, n in m[ORDER1[0]]:
                v = _out4(lambda q: m[q][i3, n], i, j, ORDER1[::-1])
                for b in range(2):
                    r0, c0 = (2 * i3 + b) * TB + QB * i, 512 * n + 128 * j
                    rest = lax.slice(partial[i3, n, b], (QB * i, 128 * j), (QB * (i + 1), 128 * (j + 1)))
                    x_s[r0:r0 + QB, c0:c0 + 128] = (_rows(v, QB * b, QB * (b + 1)) * scale + rest).astype(BF)
                    wins.append((r0, QB, c0, 128))
        for win in wins:
            send(*win)

    pacer.flush(("w2", 0))
    first = {}
    for q in ORDER1:
        if q == ORDER1[-1]:
            queue_halves(7)
        first[q] = two_levels(ORDER1[0], q)
    pacer.flush(("g", NP - 1))
    for k in range(1, 7):
        p = ORDER1[k]
        pacer.flush(("w2", k))
        if k == 2:
            split()
        if k == 6:
            pacer.flush(("f", 1, 0))
            pacer.flush(("f", 0, 1))
            send_block(1, 0)
            send_block(0, 1)
            split()
        else:
            queue_w2(k + 1)
        for c in {2: [(1, 0)], 4: [(0, 1)], 6: [(1, 1), (0, 0)]}.get(k, ()):
            queue_finish(*c)
        late = sevenths(ORDER1[0], first) if k == 1 else iter(())
        m = {}
        for q in ORDER1:
            if k == 6 and q == ORDER1[4]:
                pacer.flush(("f", 1, 1))
                pacer.flush(("f", 0, 0))
                send_last(m, [(1, 0), (0, 1)])
                send_block(1, 1)
            if k == 6 and q == ORDER1[6]:
                send_last(m, [(1, 1)])
            m[q] = three_levels(p, q, late)
        next(late, None)
        if k < 6:
            inner(p, m)
    send_last(m, [(0, 0)])
    for c in copies:
        c.wait()


@jax.jit
def pallas_sequential_preLN__sliding_block__mixer_channel_mlp__prompt_kernel(
        A_x, A_wqkv, A_wo, B_x, B_w1, B_b1, B_w2, B_b2):
    del B_x
    any_spec = pl.BlockSpec(memory_space=pl.ANY)
    out = pl.pallas_call(
        _kernel,
        out_shape=jax.ShapeDtypeStruct((S, D), BF),
        in_specs=[any_spec] * 7,
        out_specs=any_spec,
        scratch_shapes=[
            pltpu.VMEM((S, D), BF), pltpu.VMEM((D, D), BF), pltpu.VMEM((D, F), BF), pltpu.VMEM((F, D), BF),
            pltpu.VMEM((F,), BF), pltpu.VMEM((D,), BF),
            pltpu.VMEM((2 * TB, D), F32), pltpu.VMEM((512, 512), F32),
            pltpu.VMEM((3 * W, 256), I32), pltpu.VMEM((49 * S // 8, 256), I32),
            pltpu.VMEM((49 * 128 * 4, 256), I32), pltpu.VMEM((48384, 256), I32),
            pltpu.SemaphoreType.DMA((18,)), pltpu.SemaphoreType.DMA((14 * NB,)),
        ],
        compiler_params=pltpu.CompilerParams(vmem_limit_bytes=127 << 20),
        name="fused_block",
    )(A_x.reshape(S, D), A_wqkv, A_wo, B_w1, B_b1, B_w2, B_b2)
    return out.reshape(1, S, D)
```
